```python
import os as _os
_os.environ.setdefault("JAX_PLATFORMS", "cpu")
import jax
import jax.numpy as jnp

def _softmax(x, axis=-1):
    return jax.nn.softmax(x, axis=axis)
def _gelu(x):
    return jax.nn.gelu(x, approximate=True)
def _silu(x):
    return jax.nn.silu(x)
def _sigmoid(x):
    return jax.nn.sigmoid(x)
def _layernorm(x, axis=-1, eps=1e-5):
    m = jnp.mean(x, axis=axis, keepdims=True)
    v = jnp.var(x, axis=axis, keepdims=True)
    return (x - m) / jnp.sqrt(v + eps)
def _scatter_add(tgt, idx, src, axis=0):
    return tgt.at[idx].add(src)
def _segment_sum(src, seg, n):
    return jax.ops.segment_sum(src, seg, n)
class _Rng:
    def __init__(self, key):
        self._k = key
    def _next(self):
        self._k, sub = jax.random.split(self._k)
        return sub
    def normal(self, shape):
        return jax.random.normal(self._next(), shape, dtype=jnp.bfloat16)
    def randint(self, lo, hi, shape):
        return jax.random.randint(self._next(), shape, lo, hi, dtype=jnp.int32)
    def uniform(self, shape, lo=0.0, hi=1.0):
        return jax.random.uniform(self._next(), shape, jnp.bfloat16, lo, hi)
    def permutation(self, n):
        return jax.random.permutation(self._next(), n)


kernel_name = 'concat_heads__gqa_block_cached__sliding_block_cached__decode'

def setup_inputs():
    _rng = _Rng(jax.random.key(int.from_bytes(__import__("os").urandom(4), "little")))
    _w = (lambda a: (lambda t: t.astype(jnp.bfloat16) if jnp.issubdtype(t.dtype, jnp.floating) else t)(jnp.asarray(a)))
    def _A_setup():
        B, Sq, D = 2, 1, 448
        Hq, Hkv, Sk, Dh = 16, 8, 8192, 256
        assert Hq % Hkv == 0, (Hq, Hkv)
        return {
            "x": _w((lambda *s: _rng.normal(s) * 0.8)(B, Sq, D)),
            "k_cache": _w((lambda *s: _rng.normal(s) * 0.8)(B, Hkv, Sk, Dh)),
            "v_cache": _w((lambda *s: _rng.normal(s) * 0.05)(B, Hkv, Sk, Dh)),
            "wq": _w((lambda *s: _rng.normal(s) * 0.8)(D, Hq * Dh) * (D ** -0.5)),
            "wo": _w((lambda *s: _rng.normal(s) * 0.05)(Hq * Dh, D) * ((Hq * Dh) ** -0.5)),
        }
    _A_in = _A_setup()

    def _B_setup():
        B, Sq, D = 2, 1, 448
        Hq, Hkv, Sk, Dh = 16, 8, 8192, 256
        assert Hq % Hkv == 0, (Hq, Hkv)
        return {
            "x": _w((lambda *s: _rng.normal(s) * 0.8)(B, Sq, D)),
            "k_cache": _w((lambda *s: _rng.normal(s) * 0.8)(B, Hkv, Sk, Dh)),
            "v_cache": _w((lambda *s: _rng.normal(s) * 0.05)(B, Hkv, Sk, Dh)),
            "wq": _w((lambda *s: _rng.normal(s) * 0.8)(D, Hq * Dh) * (D ** -0.5)),
            "wo": _w((lambda *s: _rng.normal(s) * 0.05)(Hq * Dh, D) * ((Hq * Dh) ** -0.5)),
        }
    _B_in = _B_setup()

    return {
        "A_x": _A_in["x"],
        "A_k_cache": _A_in["k_cache"],
        "A_v_cache": _A_in["v_cache"],
        "A_wq": _A_in["wq"],
        "A_wo": _A_in["wo"],
        "B_x": _B_in["x"],
        "B_k_cache": _B_in["k_cache"],
        "B_v_cache": _B_in["v_cache"],
        "B_wq": _B_in["wq"],
        "B_wo": _B_in["wo"],
    }

def reference(A_x, A_k_cache, A_v_cache, A_wq, A_wo, B_x, B_k_cache, B_v_cache, B_wq, B_wo):
    def _A_ref(x, k_cache, v_cache, wq, wo):
        B, Sq, D = x.shape
        Hq, Dh = 16, 256
        Hkv = k_cache.shape[1]
        rep = Hq // Hkv
        q = (lambda x, *d: x.transpose(*d))((x @ wq).reshape(B, Sq, Hq, Dh), 0, 2, 1, 3)
        k = jnp.repeat(k_cache, rep, axis=1)
        v = jnp.repeat(v_cache, rep, axis=1)
        scores = jnp.einsum("bhqd,bhkd->bhqk", q, k) * (Dh ** -0.5)
        p = _softmax(scores, axis=-1)
        o = jnp.einsum("bhqk,bhkd->bhqd", p, v)
        return (lambda x, *d: x.transpose(*d))(o, 0, 2, 1, 3).reshape(B, Sq, Hq * Dh) @ wo

    def _B_ref(x, k_cache, v_cache, wq, wo):
        B, Sq, D = x.shape
        Hq, Dh = 16, 256
        Hkv, Sk = k_cache.shape[1], k_cache.shape[2]
        W = min(4096, max(256, Sk // 4))
        rep = Hq // Hkv
        q = (lambda x, *d: x.transpose(*d))((x @ wq).reshape(B, Sq, Hq, Dh), 0, 2, 1, 3)
        k = jnp.repeat(k_cache[:, :, Sk - W:, :], rep, axis=1)
        v = jnp.repeat(v_cache[:, :, Sk - W:, :], rep, axis=1)
        scores = jnp.einsum("bhqd,bhkd->bhqk", q, k) * (Dh ** -0.5)
        p = _softmax(scores, axis=-1)
        o = jnp.einsum("bhqk,bhkd->bhqd", p, v)
        return (lambda x, *d: x.transpose(*d))(o, 0, 2, 1, 3).reshape(B, Sq, Hq * Dh) @ wo

    a = _A_ref(A_x, A_k_cache, A_v_cache, A_wq, A_wo)
    b = _B_ref(B_x, B_k_cache, B_v_cache, B_wq, B_wo)
    return jnp.concatenate([a, b], axis=-1)
```

```python
import functools
import jax
import jax.numpy as jnp
from jax import lax
import jax.experimental.pallas as pl
import jax.experimental.pallas.tpu as pltpu

B, D = 2, 448
HQ, HKV, SK, DH = 16, 8, 8192, 256
REP = HQ // HKV
W = min(4096, max(256, SK // 4))
GW = REP * DH
T = 8
WG, WR = 7, 64


def _make(R=256, NBUF=3, nobc=True, do_compute=True, do_dma=True, vmem_mb=64, isplit=2):
    U = R // T
    CA = SK // R
    CB = W // R
    NA = B * CA
    NB = B * CB
    NS = NA + NB
    L = NBUF - 1
    PPB = (GW // DH) * (WR // T)
    BPG = U // PPB
    NWG = HKV // BPG
    assert U % isplit == 0 and HKV % isplit == 0

    def kernel(xa, ka, va, wqa, woa, xb, kb, vb, wqb, wob, out_ref,
               kbuf, vbuf, w_buf, x_buf, q_scr, m_scr, l_scr, acc_scr, lhs_scr,
               ksem, vsem, wsem, xsem):

        def kv_issue(src_k, src_v, b, row0, slot, u0, u1):
            if not do_dma:
                return
            for u in range(u0, u1):
                r = row0 + u * T
                if not isinstance(r, int):
                    r = pl.multiple_of(r, T)
                pltpu.make_async_copy(src_k.at[b, :, pl.ds(r, T), :],
                                      kbuf.at[slot, :, pl.ds(u * T, T), :], ksem.at[slot]).start(priority=0)
                pltpu.make_async_copy(src_v.at[b, :, pl.ds(r, T), :],
                                      vbuf.at[slot, :, pl.ds(u * T, T), :], vsem.at[slot]).start(priority=1)

        def kv_wait(slot):
            if not do_dma:
                return
            pltpu.make_async_copy(kbuf.at[slot], kbuf.at[slot], ksem.at[slot]).wait()
            pltpu.make_async_copy(vbuf.at[slot], vbuf.at[slot], vsem.at[slot]).wait()

        def w_issue(kind, p0, p1):
            if not do_dma:
                return
            srcs = (wqa, wqb) if kind == 0 else (woa, wob)
            for p in range(p0, p1):
                blk, rem = divmod(p, PPB)
                half, i = divmod(rem, WR // T)
                c0 = blk * GW + half * DH
                for br in range(2):
                    pltpu.make_async_copy(srcs[br].at[:, pl.ds(i * T, T), pl.ds(c0, DH)],
                                          w_buf.at[kind * 2 + br, :, pl.ds(i * T, T), pl.ds(c0, DH)],
                                          wsem.at[(kind * 2 + br) * HKV + blk]).start(priority=br)

        def w_wait(kind, br, blk):
            if not do_dma:
                return
            v = w_buf.at[kind * 2 + br, :, :, pl.ds(blk * GW, GW)]
            pltpu.make_async_copy(v, v, wsem.at[(kind * 2 + br) * HKV + blk]).wait()

        row = lax.broadcasted_iota(jnp.int32, (8, DH), 0)
        rowd = lax.broadcasted_iota(jnp.int32, (8, D), 0)

        cx = [pltpu.make_async_copy(xa, x_buf.at[0], xsem.at[0]),
              pltpu.make_async_copy(xb, x_buf.at[1], xsem.at[1])]

        def issue_static(g, u0, u1):
            if g < NWG:
                w_issue(0, g * U + u0, g * U + u1)
            elif g < NWG + NS:
                s = g - NWG
                if s < NA:
                    kv_issue(ka, va, s // CA, (s % CA) * R, s % NBUF, u0, u1)
                else:
                    t = s - NA
                    kv_issue(kb, vb, t // CB, SK - W + (t % CB) * R, s % NBUF, u0, u1)
            elif g < 2 * NWG + NS:
                w_issue(1, (g - NWG - NS) * U + u0, (g - NWG - NS) * U + u1)

        cx[0].start(); cx[1].start()
        for g in range(L):
            issue_static(g, 0, U)

        lhs_scr[...] = jnp.zeros(lhs_scr.shape, lhs_scr.dtype)
        cx[0].wait(); cx[1].wait()
        x8 = []
        for br in range(2):
            xv = x_buf[br].astype(jnp.float32)
            x8.append(jnp.where(rowd < 2, xv[0:1], jnp.where(rowd < 4, xv[1:2], 0.0)).astype(jnp.bfloat16))

        npart = 2 * BPG
        for g in range(NWG):
            for k in range(BPG):
                blk = g * BPG + k
                for br in range(2):
                    part = k * 2 + br
                    w_wait(0, br, blk)
                    issue_static(g + L, part * U // npart, (part + 1) * U // npart)
                    if do_compute:
                        wv = w_buf[br, :, :, blk * GW:(blk + 1) * GW].reshape(D, GW)
                        z = jnp.dot(x8[br], wv, preferred_element_type=jnp.float32)
                        qj = jnp.where(row % 2 == 0, z[:, :DH], z[:, DH:])
                        qj = qj.astype(jnp.bfloat16).astype(jnp.float32) * (DH ** -0.5)
                        q_scr[br * HKV + blk] = qj.astype(jnp.bfloat16)

        def body(s, carry):
            slot = s % NBUF
            is_a = s < NA
            t = jnp.where(is_a, s, s - NA)
            b = jnp.where(is_a, t // CA, t // CB)
            c = t - b * jnp.where(is_a, CA, CB)
            first = c == 0
            last = c == jnp.where(is_a, CA, CB) - 1
            br = jnp.where(is_a, 0, 1)

            g = s + L
            gslot = g % NBUF
            g_a = g < NA
            g_b = jnp.logical_and(g >= NA, g < NS)
            ga = jnp.minimum(g, NA - 1)
            gb = jnp.clip(g - NA, 0, NB - 1)

            def issue_part(u0, u1):
                @pl.when(g_a)
                def _():
                    kv_issue(ka, va, ga // CA, (ga % CA) * R, gslot, u0, u1)

                @pl.when(g_b)
                def _():
                    kv_issue(kb, vb, gb // CB, SK - W + (gb % CB) * R, gslot, u0, u1)

                for k in range(L):
                    @pl.when(g == NS + k)
                    def _():
                        w_issue(1, k * U + u0, k * U + u1)

            kv_wait(slot)

            if do_compute:
                @pl.when(first)
                def _():
                    m_scr[...] = jnp.full(m_scr.shape, -jnp.inf, jnp.float32)
                    l_scr[...] = jnp.zeros(l_scr.shape, jnp.float32)
                    acc_scr[...] = jnp.zeros(acc_scr.shape, jnp.float32)

            hp = HKV // isplit
            for part in range(isplit):
                issue_part(part * U // isplit, (part + 1) * U // isplit)
                if not do_compute:
                    continue
                for j in range(part * hp, (part + 1) * hp):
                    q = q_scr[br * HKV + j]
                    sc = lax.dot_general(q, kbuf[slot, j], (((1,), (1,)), ((), ())),
                                         preferred_element_type=jnp.float32)
                    m_prev = m_scr[j]
                    m_new = jnp.maximum(m_prev, jnp.max(sc, axis=1, keepdims=True))
                    alpha = jnp.exp(m_prev - m_new)
                    p = jnp.exp(sc - jnp.concatenate([m_new] * (R // 128), axis=1))
                    psum = p[:, 0:128]
                    for i in range(1, R // 128):
                        psum = psum + p[:, i * 128:(i + 1) * 128]
                    m_scr[j] = m_new
                    l_scr[j] = alpha * l_scr[j] + psum
                    pv = jnp.dot(p.astype(jnp.bfloat16), vbuf[slot, j], preferred_element_type=jnp.float32)
                    acc_scr[j] = jnp.concatenate([alpha, alpha], axis=1) * acc_scr[j] + pv

            if do_compute:
                @pl.when(last)
                def _():
                    for j in range(HKV):
                        l = jnp.sum(l_scr[j], axis=1, keepdims=True)
                        o = (acc_scr[j] / l)
                        old = lhs_scr[br * HKV + j].astype(jnp.float32)
                        new = jnp.concatenate([jnp.where(row == 2 * b, o, old[:, :DH]),
                                               jnp.where(row == 2 * b + 1, o, old[:, DH:])], axis=1)
                        lhs_scr[br * HKV + j] = new.astype(jnp.bfloat16)
            return carry

        lax.fori_loop(0, NS, body, 0)

        y = [jnp.zeros((8, D), jnp.float32), jnp.zeros((8, D), jnp.float32)]
        for g in range(NWG):
            for k in range(BPG):
                blk = g * BPG + k
                for br in range(2):
                    part = k * 2 + br
                    w_wait(1, br, blk)
                    issue_static(NWG + NS + g + L, part * U // npart, (part + 1) * U // npart)
                    if do_compute:
                        wv = w_buf[2 + br, :, :, blk * GW:(blk + 1) * GW].reshape(D, GW)
                        y[br] = y[br] + lax.dot_general(lhs_scr[br * HKV + blk], wv, (((1,), (1,)), ((), ())),
                                                        preferred_element_type=jnp.float32)
        for br in range(2):
            yy = y[br]
            res = jnp.concatenate([yy[0:1] + yy[1:2], yy[2:3] + yy[3:4]], axis=0)
            out_ref[:, br * D:(br + 1) * D] = res.astype(out_ref.dtype)

    @jax.jit
    def fn(A_x, A_k_cache, A_v_cache, A_wq, A_wo, B_x, B_k_cache, B_v_cache, B_wq, B_wo):
        hbm = pl.BlockSpec(memory_space=pltpu.HBM)
        def prep(x, k, v, wq, wo):
            return (x.reshape(B, D), k, v, wq.reshape(WG, WR, HQ * DH), wo.T.reshape(WG, WR, HQ * DH))
        out = pl.pallas_call(
            kernel,
            out_shape=jax.ShapeDtypeStruct((B, 2 * D), jnp.bfloat16),
            in_specs=[hbm] * 10,
            out_specs=pl.BlockSpec(memory_space=pltpu.VMEM),
            scratch_shapes=[
                pltpu.VMEM((NBUF, HKV, R, DH), jnp.bfloat16),
                pltpu.VMEM((NBUF, HKV, R, DH), jnp.bfloat16),
                pltpu.VMEM((4, WG, WR, HQ * DH), jnp.bfloat16),
                pltpu.VMEM((2, B, D), jnp.bfloat16),
                pltpu.VMEM((2 * HKV, 8, DH), jnp.bfloat16),
                pltpu.VMEM((HKV, 8, 128), jnp.float32),
                pltpu.VMEM((HKV, 8, 128), jnp.float32),
                pltpu.VMEM((HKV, 8, DH), jnp.float32),
                pltpu.VMEM((2 * HKV, 8, GW), jnp.bfloat16),
                pltpu.SemaphoreType.DMA((NBUF,)),
                pltpu.SemaphoreType.DMA((NBUF,)),
                pltpu.SemaphoreType.DMA((4 * HKV,)),
                pltpu.SemaphoreType.DMA((2,)),
            ],
            compiler_params=pltpu.CompilerParams(vmem_limit_bytes=vmem_mb * 1024 * 1024,
                                                 disable_bounds_checks=nobc),
        )(*prep(A_x, A_k_cache, A_v_cache, A_wq, A_wo), *prep(B_x, B_k_cache, B_v_cache, B_wq, B_wo))
        return out.reshape(B, 1, 2 * D)
    return fn


pallas_concat_heads__gqa_block_cached__sliding_block_cached__decode_kernel = _make()
```

```python
import jax
import jax.numpy as jnp
from jax import lax
import jax.experimental.pallas as pl
import jax.experimental.pallas.tpu as pltpu

B, D = 2, 448
HQ, HKV, SK, DH = 16, 8, 8192, 256
REP = HQ // HKV
W = min(4096, max(256, SK // 4))
GW = REP * DH
NQ = HQ * DH

T = 8
R = 256
U = R // T
NBUF = 3
LEADG = NBUF - 1
LEAD = LEADG * U
CA, CB = SK // R, W // R
NA, NB = B * CA, B * CB
NS = NA + NB
ISPLIT = 2

WG, WR, WC = 4, 112, 512
NWC = NQ // WC
NWI = WR // T
NWP = NWI * NWC


def _stream_plan(blocks, last_split=None):
    segs, dmas = [], []
    i0 = 0
    for n, nb in enumerate(blocks):
        i1 = i0 + nb
        if n == len(blocks) - 1 and last_split is not None:
            c0 = 0
            for c1 in last_split:
                dmas += [(i, c, len(segs)) for c in range(c0, c1) for i in range(i0, i1)]
                segs.append((i0, i1, c0, c1))
                c0 = c1
            assert c0 == NWC
        else:
            dmas += [(i, c, len(segs)) for i in range(i0, i1) for c in range(NWC)]
            segs.append((i0, i1, 0, NWC))
        i0 = i1
    assert i0 == NWI and len(dmas) == NWP
    return segs, dmas


PLANS = (
    _stream_plan((4, 4, 4, 2)),
    _stream_plan((4, 4, 4, 2)),
    _stream_plan((4, 4, 4, 2)),
    _stream_plan((4, 4, 2, 2, 2), (4, 8)),
)
SEM_BASE = [0]
for _p in PLANS:
    SEM_BASE.append(SEM_BASE[-1] + len(_p[0]))
O_ORDER = ((0, 0), (1, 0), (0, 1), (1, 1), (0, 2), (1, 2), (0, 3), (1, 3), (1, 4), (1, 5))
O_ISSUE = (16, 16, 16)

_NT = (((1,), (1,)), ((), ()))


def _kernel(xa, ka, va, wqa, woa, xb, kb, vb, wqb, wob, out_ref,
            kbuf, vbuf, w_buf, x_buf, q_scr, z_scr, m_scr, l_scr, acc_scr, lhs_scr,
            ksem, vsem, wsem, xsem):
    w_src = (wqa, wqb, woa, wob)

    def kv_issue(src_k, src_v, b, row0, slot, u0, u1):
        for u in range(u0, u1):
            r = row0 + u * T
            if not isinstance(r, int):
                r = pl.multiple_of(r, T)
            pltpu.make_async_copy(src_k.at[b, :, pl.ds(r, T), :],
                                  kbuf.at[slot, :, pl.ds(u * T, T), :],
                                  ksem.at[slot]).start(priority=0)
            pltpu.make_async_copy(src_v.at[b, :, pl.ds(r, T), :],
                                  vbuf.at[slot, :, pl.ds(u * T, T), :],
                                  vsem.at[slot]).start(priority=1)

    def kv_wait(slot):
        pltpu.make_async_copy(kbuf.at[slot], kbuf.at[slot], ksem.at[slot]).wait()
        pltpu.make_async_copy(vbuf.at[slot], vbuf.at[slot], vsem.at[slot]).wait()

    def w_issue(kind, p0, p1):
        for p in range(p0, min(p1, NWP)):
            for br in range(2):
                m = kind * 2 + br
                i, c, seg = PLANS[m][1][p]
                pltpu.make_async_copy(w_src[m].at[:, pl.ds(i * T, T), pl.ds(c * WC, WC)],
                                      w_buf.at[m, :, pl.ds(i * T, T), pl.ds(c * WC, WC)],
                                      wsem.at[SEM_BASE[m] + seg]).start(priority=br)

    def w_wait(m, seg):
        i0, i1, c0, c1 = PLANS[m][0][seg]
        v = w_buf.at[m, :, pl.ds(i0 * T, (i1 - i0) * T), pl.ds(c0 * WC, (c1 - c0) * WC)]
        pltpu.make_async_copy(v, v, wsem.at[SEM_BASE[m] + seg]).wait()

    def w_load(m, seg):
        i0, i1, c0, c1 = PLANS[m][0][seg]
        blk = w_buf[m, :, i0 * T:i1 * T, c0 * WC:c1 * WC]
        return blk.reshape(WG * (i1 - i0) * T, (c1 - c0) * WC)

    def issue_head(p0, p1):
        for p in range(p0, p1):
            if p < NWP:
                w_issue(0, p, p + 1)
            else:
                s, u = divmod(p - NWP, U)
                kv_issue(ka, va, s // CA, (s % CA) * R, s % NBUF, u, u + 1)

    row = lax.broadcasted_iota(jnp.int32, (8, DH), 0)
    rowd = lax.broadcasted_iota(jnp.int32, (8, D), 0)

    cx = [pltpu.make_async_copy(xa, x_buf.at[0], xsem.at[0]),
          pltpu.make_async_copy(xb, x_buf.at[1], xsem.at[1])]
    issue_head(0, 4)
    cx[0].start()
    cx[1].start()
    pos = LEAD
    issue_head(4, pos)

    lhs_scr[...] = jnp.zeros(lhs_scr.shape, lhs_scr.dtype)
    cx[0].wait()
    cx[1].wait()
    x8 = []
    for br in range(2):
        xv = x_buf[br].astype(jnp.float32)
        x8.append(jnp.where(rowd < 2, xv[0:1], jnp.where(rowd < 4, xv[1:2], 0.0)))

    target = NWP + LEAD
    nparts = 2 * len(PLANS[0][0]) - 1
    for seg, (i0, i1, _, _) in enumerate(PLANS[0][0]):
        for br in range(2):
            part = 2 * seg + br
            w_wait(br, seg)
            nxt = min(target, LEAD + (part + 1) * (NWP + nparts - 1) // nparts)
            issue_head(pos, nxt)
            pos = nxt
            xk = jnp.concatenate(
                [x8[br][:, g * WR + i0 * T:g * WR + i1 * T] for g in range(WG)], axis=1)
            z = jnp.dot(xk.astype(jnp.bfloat16), w_load(br, seg),
                        preferred_element_type=jnp.float32)
            if i0 > 0:
                z = z + z_scr[br]
            if i1 < NWI:
                z_scr[br] = z
            else:
                for j in range(HKV):
                    qj = jnp.where(row % 2 == 0, z[:, j * GW:j * GW + DH],
                                   z[:, j * GW + DH:(j + 1) * GW])
                    qj = qj.astype(jnp.bfloat16).astype(jnp.float32) * (DH ** -0.5)
                    q_scr[br * HKV + j] = qj.astype(jnp.bfloat16)
    assert pos == target

    def body(s, carry):
        slot = s % NBUF
        is_a = s < NA
        t = jnp.where(is_a, s, s - NA)
        b = jnp.where(is_a, t // CA, t // CB)
        cn = jnp.where(is_a, CA, CB)
        c = t - b * cn
        br = jnp.where(is_a, 0, 1)

        g = s + LEADG
        gslot = g % NBUF
        ga = jnp.minimum(g, NA - 1)
        gb = jnp.clip(g - NA, 0, NB - 1)

        def issue_part(u0, u1):
            @pl.when(g < NA)
            def _():
                kv_issue(ka, va, ga // CA, (ga % CA) * R, gslot, u0, u1)

            @pl.when(jnp.logical_and(g >= NA, g < NS))
            def _():
                kv_issue(kb, vb, gb // CB, SK - W + (gb % CB) * R, gslot, u0, u1)

            for k in range(LEADG):
                @pl.when(g == NS + k)
                def _():
                    w_issue(1, k * U + u0, k * U + u1)

        kv_wait(slot)

        @pl.when(c == 0)
        def _():
            m_scr[...] = jnp.full(m_scr.shape, -jnp.inf, jnp.float32)
            l_scr[...] = jnp.zeros(l_scr.shape, jnp.float32)
            acc_scr[...] = jnp.zeros(acc_scr.shape, jnp.float32)

        hp = HKV // ISPLIT
        for part in range(ISPLIT):
            issue_part(part * U // ISPLIT, (part + 1) * U // ISPLIT)
            for j in range(part * hp, (part + 1) * hp):
                q = q_scr[br * HKV + j]
                sc = lax.dot_general(q, kbuf[slot, j], _NT,
                                     preferred_element_type=jnp.float32)
                m_prev = m_scr[j]
                m_new = jnp.maximum(m_prev, jnp.max(sc, axis=1, keepdims=True))
                alpha = jnp.exp(m_prev - m_new)
                p = jnp.exp(sc - jnp.concatenate([m_new] * (R // 128), axis=1))
                psum = p[:, 0:128]
                for i in range(1, R // 128):
                    psum = psum + p[:, i * 128:(i + 1) * 128]
                m_scr[j] = m_new
                l_scr[j] = alpha * l_scr[j] + psum
                pv = jnp.dot(p.astype(jnp.bfloat16), vbuf[slot, j],
                             preferred_element_type=jnp.float32)
                acc_scr[j] = jnp.concatenate([alpha] * (DH // 128), axis=1) * acc_scr[j] + pv

        @pl.when(c == cn - 1)
        def _():
            for j in range(HKV):
                o = acc_scr[j] / jnp.sum(l_scr[j], axis=1, keepdims=True)
                old = lhs_scr[br, :, j * GW:(j + 1) * GW].astype(jnp.float32)
                new = jnp.concatenate(
                    [jnp.where(row == 2 * b, o, old[:, :DH]),
                     jnp.where(row == 2 * b + 1, o, old[:, DH:])], axis=1)
                lhs_scr[br, :, j * GW:(j + 1) * GW] = new.astype(jnp.bfloat16)

        return carry

    lax.fori_loop(0, NS, body, 0)

    wpos = LEAD
    ypart = [None, None]
    for n, (br, seg) in enumerate(O_ORDER):
        m = 2 + br
        i0, i1, c0, c1 = PLANS[m][0][seg]
        assert max(p for p, d in enumerate(PLANS[m][1]) if d[2] == seg) < wpos
        w_wait(m, seg)
        if n < len(O_ISSUE):
            w_issue(1, wpos, wpos + O_ISSUE[n])
            wpos += O_ISSUE[n]
        y = lax.dot_general(lhs_scr[br, :, c0 * WC:c1 * WC], w_load(m, seg), _NT,
                            preferred_element_type=jnp.float32)
        if c0 > 0:
            y = y + ypart[br]
        if c1 < NWC:
            ypart[br] = y
            continue
        nr = (i1 - i0) * T
        res = jnp.concatenate([y[0:1] + y[1:2], y[2:3] + y[3:4]], axis=0)
        res = res.astype(out_ref.dtype)
        for g in range(WG):
            o0 = br * D + g * WR + i0 * T
            out_ref[:, o0:o0 + nr] = res[:, g * nr:(g + 1) * nr]
    assert wpos == NWP


@jax.jit
def pallas_concat_heads__gqa_block_cached__sliding_block_cached__decode_kernel(
    A_x: jax.Array,
    A_k_cache: jax.Array,
    A_v_cache: jax.Array,
    A_wq: jax.Array,
    A_wo: jax.Array,
    B_x: jax.Array,
    B_k_cache: jax.Array,
    B_v_cache: jax.Array,
    B_wq: jax.Array,
    B_wo: jax.Array,
):
    assert A_x.shape == B_x.shape == (B, 1, D)
    assert A_k_cache.shape == A_v_cache.shape == (B, HKV, SK, DH)
    assert B_k_cache.shape == B_v_cache.shape == (B, HKV, SK, DH)
    assert A_wq.shape == B_wq.shape == (D, NQ)
    assert A_wo.shape == B_wo.shape == (NQ, D)

    def prep(x, k, v, wq, wo):
        return (x.reshape(B, D), k, v, wq.reshape(WG, WR, NQ), wo.T.reshape(WG, WR, NQ))

    bf16, f32 = jnp.bfloat16, jnp.float32
    out = pl.pallas_call(
        _kernel,
        out_shape=jax.ShapeDtypeStruct((B, 2 * D), bf16),
        in_specs=[pl.BlockSpec(memory_space=pltpu.HBM)] * 10,
        out_specs=pl.BlockSpec(memory_space=pltpu.VMEM),
        scratch_shapes=[
            pltpu.VMEM((NBUF, HKV, R, DH), bf16),
            pltpu.VMEM((NBUF, HKV, R, DH), bf16),
            pltpu.VMEM((4, WG, WR, NQ), bf16),
            pltpu.VMEM((2, B, D), bf16),
            pltpu.VMEM((2 * HKV, 8, DH), bf16),
            pltpu.VMEM((2, 8, NQ), f32),
            pltpu.VMEM((HKV, 8, 128), f32),
            pltpu.VMEM((HKV, 8, 128), f32),
            pltpu.VMEM((HKV, 8, DH), f32),
            pltpu.VMEM((2, 8, NQ), bf16),
            pltpu.SemaphoreType.DMA((NBUF,)),
            pltpu.SemaphoreType.DMA((NBUF,)),
            pltpu.SemaphoreType.DMA((SEM_BASE[-1],)),
            pltpu.SemaphoreType.DMA((2,)),
        ],
        compiler_params=pltpu.CompilerParams(
            vmem_limit_bytes=64 * 1024 * 1024,
            disable_bounds_checks=True,
            disable_semaphore_checks=True,
        ),
    )(*prep(A_x, A_k_cache, A_v_cache, A_wq, A_wo),
      *prep(B_x, B_k_cache, B_v_cache, B_wq, B_wo))
    return out.reshape(B, 1, 2 * D)
```

```python
import contextlib
import jax
import jax.numpy as jnp
from jax import lax
import jax.experimental.pallas as pl
import jax.experimental.pallas.tpu as pltpu

B, D = 2, 448
HQ, HKV, SK, DH = 16, 8, 8192, 256
REP = HQ // HKV
W = min(4096, max(256, SK // 4))
GW = REP * DH
NQ = HQ * DH

T = 8
R = 256
U = R // T
NBUF = 3
LEADG = NBUF - 1
LEAD = LEADG * U
CA, CB = SK // R, W // R
NA, NB = B * CA, B * CB
NS = NA + NB
ISPLIT = 2

WG, WR, WC = 4, 112, 512
NWC = NQ // WC
NWI = WR // T
NWP = NWI * NWC
SEGI = 2
SEGR = SEGI * T
NSEG = NWI // SEGI
SEGP = SEGI * NWC

_NT = (((1,), (1,)), ((), ()))


def make(unroll=4, scopes=False, o_sched=None, q_lag=0, nobc=True, nosc=True, OI=8, asm_back=1, n_static=2, tail=(4, 6, 8)):
    def scope(name):
        return jax.named_scope(name) if scopes else contextlib.nullcontext()

    if o_sched is None:
        o_sched = [(0, 0), (0, 1), (1, 0), (0, 2), (1, 1), (0, 3), (1, 2), (0, 4), (1, 3), (0, 5), (1, 4), (0, 6), (1, 5), (1, 6)]
    assert sorted(o_sched) == sorted((br, s) for br in range(2) for s in range(NSEG))

    def kernel(xa, ka, va, wqa, woa, xb, kb, vb, wqb, wob, out_ref,
               kbuf, vbuf, w_buf, x_buf, xk_scr, q_scr, z_scr, m_scr, l_scr, acc_scr, lhs_scr, y_scr,
               ksem, vsem, wsem, xsem):
        w_src = (wqa, wqb, woa, wob)

        def kv_issue(src_k, src_v, b, row0, slot, u0, n, kv_unroll=True):
            def one(k, carry):
                u = u0 + k
                r = pl.multiple_of(row0 + u * T, T)
                d = pl.multiple_of(u * T, T)
                pltpu.make_async_copy(src_k.at[b, :, pl.ds(r, T), :], kbuf.at[slot, :, pl.ds(d, T), :],
                                      ksem.at[slot]).start(priority=0)
                pltpu.make_async_copy(src_v.at[b, :, pl.ds(r, T), :], vbuf.at[slot, :, pl.ds(d, T), :],
                                      vsem.at[slot]).start(priority=1)
                return carry
            if kv_unroll:
                for k in range(n):
                    one(k, 0)
            else:
                lax.fori_loop(0, n, one, 0, unroll=unroll)

        def kv_wait(slot):
            pltpu.make_async_copy(kbuf.at[slot], kbuf.at[slot], ksem.at[slot]).wait()
            pltpu.make_async_copy(vbuf.at[slot], vbuf.at[slot], vsem.at[slot]).wait()

        def w_issue(kind, p0, n):
            def one(k, carry):
                p = p0 + k
                r = pl.multiple_of((p // NWC) * T, T)
                c = pl.multiple_of((p % NWC) * WC, WC)
                for br in range(2):
                    m = kind * 2 + br
                    pltpu.make_async_copy(w_src[m].at[:, pl.ds(r, T), pl.ds(c, WC)],
                                          w_buf.at[m, :, pl.ds(r, T), pl.ds(c, WC)],
                                          wsem.at[m * NSEG + p // SEGP]).start(priority=br)
                return carry
            lax.fori_loop(0, n, one, 0, unroll=unroll)

        def w_wait(m, seg):
            v = w_buf.at[m, :, pl.ds(pl.multiple_of(seg * SEGR, SEGR), SEGR), :]
            pltpu.make_async_copy(v, v, wsem.at[m * NSEG + seg]).wait()

        def w_load(m, seg, n=1):
            blk = w_buf[m, :, pl.ds(pl.multiple_of(seg * SEGR, SEGR), n * SEGR), :]
            return blk.reshape(WG * n * SEGR, NQ)

        row = lax.broadcasted_iota(jnp.int32, (8, DH), 0)
        rowd = lax.broadcasted_iota(jnp.int32, (8, D), 0)

        cx = [pltpu.make_async_copy(xa, x_buf.at[0], xsem.at[0]),
              pltpu.make_async_copy(xb, x_buf.at[1], xsem.at[1])]
        w_issue(0, 0, 4)
        cx[0].start(); cx[1].start()
        w_issue(0, 4, LEAD - 4)

        lhs_scr[...] = jnp.zeros(lhs_scr.shape, lhs_scr.dtype)
        z_scr[...] = jnp.zeros(z_scr.shape, z_scr.dtype)
        cx[0].wait(); cx[1].wait()
        for br in range(2):
            xv = x_buf[br].astype(jnp.float32)
            x8 = jnp.where(rowd < 2, xv[0:1], jnp.where(rowd < 4, xv[1:2], 0.0))
            for seg in range(NSEG):
                xk_scr[br * NSEG + seg] = jnp.concatenate(
                    [x8[:, g * WR + seg * SEGR:g * WR + (seg + 1) * SEGR] for g in range(WG)],
                    axis=1).astype(jnp.bfloat16)

        QI = NWP // (2 * NSEG)

        def qbody(it, carry):
            seg = it // 2
            br = it % 2
            w_wait(br, seg)
            p = LEAD + it * QI

            @pl.when(p < NWP)
            def _():
                w_issue(0, jnp.minimum(p, NWP - QI), QI)

            @pl.when(p >= NWP)
            def _():
                u = jnp.maximum(p - NWP, 0)
                s = u // U
                kv_issue(ka, va, 0, s * R, s, u - s * U, QI, kv_unroll=False)

            z_scr[br] += jnp.dot(xk_scr[br * NSEG + seg], w_load(br, seg), preferred_element_type=jnp.float32)
            return carry

        with scope("qloop"):
            lax.fori_loop(0, 2 * NSEG, qbody, 0)

        def qfin(n, carry):
            br = n // HKV
            j = n % HKV
            z = z_scr[br, :, pl.ds(pl.multiple_of(j * GW, GW), GW)]
            qj = jnp.where(row % 2 == 0, z[:, :DH], z[:, DH:])
            qj = qj.astype(jnp.bfloat16).astype(jnp.float32) * (DH ** -0.5)
            q_scr[n] = qj.astype(jnp.bfloat16)
            return carry
        lax.fori_loop(0, 2 * HKV, qfin, 0)

        def body(s, carry):
            slot = s % NBUF
            is_a = s < NA
            t = jnp.where(is_a, s, s - NA)
            b = jnp.where(is_a, t // CA, t // CB)
            cn = jnp.where(is_a, CA, CB)
            c = t - b * cn
            br = jnp.where(is_a, 0, 1)

            g = s + LEADG
            gslot = g % NBUF
            ga = jnp.minimum(g, NA - 1)
            gb = jnp.clip(g - NA, 0, NB - 1)
            gw = jnp.maximum(g - NS, 0)

            def issue_part(u0, n):
                @pl.when(g < NA)
                def _():
                    kv_issue(ka, va, ga // CA, (ga % CA) * R, gslot, u0, n)

                @pl.when(jnp.logical_and(g >= NA, g < NS))
                def _():
                    kv_issue(kb, vb, gb // CB, SK - W + (gb % CB) * R, gslot, u0, n)

                @pl.when(g >= NS)
                def _():
                    w_issue(1, gw * U + u0, n)

            kv_wait(slot)

            @pl.when(c == 0)
            def _():
                m_scr[...] = jnp.full(m_scr.shape, -jnp.inf, jnp.float32)
                l_scr[...] = jnp.zeros(l_scr.shape, jnp.float32)
                acc_scr[...] = jnp.zeros(acc_scr.shape, jnp.float32)

            hp = HKV // ISPLIT
            for part in range(ISPLIT):
                issue_part(part * U // ISPLIT, U // ISPLIT)
                for j in range(part * hp, (part + 1) * hp):
                    q = q_scr[br * HKV + j]
                    sc = lax.dot_general(q, kbuf[slot, j], _NT, preferred_element_type=jnp.float32)
                    m_prev = m_scr[j]
                    m_new = jnp.maximum(m_prev, jnp.max(sc, axis=1, keepdims=True))
                    alpha = jnp.exp(m_prev - m_new)
                    p = jnp.exp(sc - jnp.concatenate([m_new] * (R // 128), axis=1))
                    psum = p[:, 0:128]
                    for i in range(1, R // 128):
                        psum = psum + p[:, i * 128:(i + 1) * 128]
                    m_scr[j] = m_new
                    l_scr[j] = alpha * l_scr[j] + psum
                    pv = jnp.dot(p.astype(jnp.bfloat16), vbuf[slot, j], preferred_element_type=jnp.float32)
                    acc_scr[j] = jnp.concatenate([alpha] * (DH // 128), axis=1) * acc_scr[j] + pv

            @pl.when(c == cn - 1)
            def _():
                for j in range(HKV):
                    o = acc_scr[j] / jnp.sum(l_scr[j], axis=1, keepdims=True)
                    old = lhs_scr[br, :, j * GW:(j + 1) * GW].astype(jnp.float32)
                    new = jnp.concatenate(
                        [jnp.where(row == 2 * b, o, old[:, :DH]),
                         jnp.where(row == 2 * b + 1, o, old[:, DH:])], axis=1)
                    lhs_scr[br, :, j * GW:(j + 1) * GW] = new.astype(jnp.bfloat16)
            return carry

        with scope("kvloop"):
            lax.fori_loop(0, NS, body, 0)

        def emit(br, seg, y):
            res = jnp.concatenate([y[0:1] + y[1:2], y[2:3] + y[3:4]], axis=0).astype(out_ref.dtype)
            for g in range(WG):
                o0 = br * D + g * WR + seg * SEGR
                out_ref[:, o0:o0 + SEGR] = res[:, g * SEGR:(g + 1) * SEGR]

        def sel(it, vals):
            out = jnp.int32(vals[0])
            for k in range(1, len(vals)):
                out = jnp.where(it >= k, jnp.int32(vals[k]), out)
            return out

        NL = 2 * NSEG - n_static
        assert o_sched[-1] == (1, NSEG - 1)
        n_oi = (NWP - SEGP - LEAD) // OI
        for it, (br, seg) in enumerate(o_sched):
            issued = LEAD + min(it, n_oi) * OI + (SEGP if it > n_oi else 0)
            assert (seg + 1) * SEGP <= issued, (it, br, seg)

        def issue_last():
            la = [(i, c) for i in range(NWI - SEGI, NWI) for c in range(NWC)]
            lb, c0 = [], 0
            for t, c1 in enumerate(tail):
                lb += [(i, c, t) for i in range(NWI - SEGI, NWI) for c in range(c0, c1)]
                c0 = c1
            for (ia, ca), (ib, cb, t) in zip(la, lb):
                pltpu.make_async_copy(woa.at[:, pl.ds(ia * T, T), pl.ds(ca * WC, WC)],
                                      w_buf.at[2, :, pl.ds(ia * T, T), pl.ds(ca * WC, WC)],
                                      wsem.at[3 * NSEG - 1]).start(priority=0)
                pltpu.make_async_copy(wob.at[:, pl.ds(ib * T, T), pl.ds(cb * WC, WC)],
                                      w_buf.at[3, :, pl.ds(ib * T, T), pl.ds(cb * WC, WC)],
                                      wsem.at[4 * NSEG - 1 + t]).start(priority=1)

        def obody(it, carry):
            br = sel(it, [x[0] for x in o_sched[:NL]])
            seg = sel(it, [x[1] for x in o_sched[:NL]])
            with scope("ow"):
                w_wait(2 + br, seg)

            @pl.when(it < n_oi)
            def _():
                w_issue(1, LEAD + jnp.minimum(it, n_oi - 1) * OI, OI)

            @pl.when(it == n_oi)
            def _():
                issue_last()

            with scope("oc"):
                y_scr[br * NSEG + seg] = lax.dot_general(lhs_scr[br], w_load(2 + br, seg), _NT,
                                                         preferred_element_type=jnp.float32)

            @pl.when(it == NL - 1 - asm_back)
            def _():
                for (b2, s2) in o_sched[:NL - asm_back]:
                    emit(b2, s2, y_scr[b2 * NSEG + s2])
            return carry

        with scope("oloop"):
            lax.fori_loop(0, NL, obody, 0)
        with scope("asm"):
            for (b2, s2) in o_sched[NL - asm_back:NL]:
                emit(b2, s2, y_scr[b2 * NSEG + s2])
        for (b2, s2) in o_sched[NL:-1]:
            with scope("sw"):
                w_wait(2 + b2, s2)
            with scope("sc"):
                emit(b2, s2, lax.dot_general(lhs_scr[b2], w_load(2 + b2, s2), _NT,
                                             preferred_element_type=jnp.float32))
        y, c0 = None, 0
        r0 = (NSEG - 1) * SEGR
        for t, c1 in enumerate(tail):
            v = w_buf.at[3, :, pl.ds(r0, SEGR), pl.ds(c0 * WC, (c1 - c0) * WC)]
            with scope("tw"):
                pltpu.make_async_copy(v, v, wsem.at[4 * NSEG - 1 + t]).wait()
            with scope("tc"):
                blk = w_buf[3, :, r0:r0 + SEGR, c0 * WC:c1 * WC].reshape(WG * SEGR, (c1 - c0) * WC)
                yy = lax.dot_general(lhs_scr[1, :, c0 * WC:c1 * WC], blk, _NT, preferred_element_type=jnp.float32)
                y = yy if y is None else y + yy
                if c1 == NWC:
                    emit(1, NSEG - 1, y)
            c0 = c1

    @jax.jit
    def fn(A_x, A_k_cache, A_v_cache, A_wq, A_wo, B_x, B_k_cache, B_v_cache, B_wq, B_wo):
        def prep(x, k, v, wq, wo):
            return (x.reshape(B, D), k, v, wq.reshape(WG, WR, NQ), wo.T.reshape(WG, WR, NQ))
        bf16, f32 = jnp.bfloat16, jnp.float32
        out = pl.pallas_call(
            kernel,
            out_shape=jax.ShapeDtypeStruct((B, 2 * D), bf16),
            in_specs=[pl.BlockSpec(memory_space=pltpu.HBM)] * 10,
            out_specs=pl.BlockSpec(memory_space=pltpu.VMEM),
            scratch_shapes=[
                pltpu.VMEM((NBUF, HKV, R, DH), bf16),
                pltpu.VMEM((NBUF, HKV, R, DH), bf16),
                pltpu.VMEM((4, WG, WR, NQ), bf16),
                pltpu.VMEM((2, B, D), bf16),
                pltpu.VMEM((2 * NSEG, 8, WG * SEGR), bf16),
                pltpu.VMEM((2 * HKV, 8, DH), bf16),
                pltpu.VMEM((2, 8, NQ), f32),
                pltpu.VMEM((HKV, 8, 128), f32),
                pltpu.VMEM((HKV, 8, 128), f32),
                pltpu.VMEM((HKV, 8, DH), f32),
                pltpu.VMEM((2, 8, NQ), bf16),
                pltpu.VMEM((2 * NSEG, 8, WG * SEGR), f32),
                pltpu.SemaphoreType.DMA((NBUF,)),
                pltpu.SemaphoreType.DMA((NBUF,)),
                pltpu.SemaphoreType.DMA((4 * NSEG - 1 + len(tail),)),
                pltpu.SemaphoreType.DMA((2,)),
            ],
            compiler_params=pltpu.CompilerParams(
                vmem_limit_bytes=64 * 1024 * 1024,
                disable_bounds_checks=nobc,
                disable_semaphore_checks=nosc,
            ),
        )(*prep(A_x, A_k_cache, A_v_cache, A_wq, A_wo),
          *prep(B_x, B_k_cache, B_v_cache, B_wq, B_wo))
        return out.reshape(B, 1, 2 * D)
    return fn


pallas_concat_heads__gqa_block_cached__sliding_block_cached__decode_kernel = make(**dict(n_static=1, asm_back=2))
```

```python
import contextlib
import jax
import jax.numpy as jnp
from jax import lax
import jax.experimental.pallas as pl
import jax.experimental.pallas.tpu as pltpu

B, D = 2, 448
HQ, HKV, SK, DH = 16, 8, 8192, 256
REP = HQ // HKV
W = min(4096, max(256, SK // 4))
GW = REP * DH
NQ = HQ * DH

T = 8
R = 256
U = R // T
NBUF = 3
LEADG = NBUF - 1
LEAD = LEADG * U
CA, CB = SK // R, W // R
NA, NB = B * CA, B * CB
NS = NA + NB
ISPLIT = 2

WG, WR, WC = 4, 112, 512
NWC = NQ // WC
NWI = WR // T
NWP = NWI * NWC
SEGI = 2
SEGR = SEGI * T
NSEG = NWI // SEGI
SEGP = SEGI * NWC

_NT = (((1,), (1,)), ((), ()))


def make(unroll=4, scopes=False, o_sched=None, q_lag=0, nobc=True, nosc=True, asm_at=2, OI=8):
    def scope(name):
        return jax.named_scope(name) if scopes else contextlib.nullcontext()

    if o_sched is None:
        o_sched = [(0, 0), (0, 1), (1, 0), (0, 2), (1, 1), (0, 3), (1, 2), (0, 4), (1, 3), (0, 5), (1, 4), (0, 6), (1, 5), (1, 6)]
    assert sorted(o_sched) == sorted((br, s) for br in range(2) for s in range(NSEG))

    def kernel(xa, ka, va, wqa, woa, xb, kb, vb, wqb, wob, out_ref,
               kbuf, vbuf, w_buf, x_buf, xk_scr, q_scr, z_scr, m_scr, l_scr, acc_scr, lhs_scr, y_scr,
               ksem, vsem, wsem, xsem):
        w_src = (wqa, wqb, woa, wob)

        def kv_issue(src_k, src_v, b, row0, slot, u0, n, kv_unroll=True):
            def one(k, carry):
                u = u0 + k
                r = pl.multiple_of(row0 + u * T, T)
                d = pl.multiple_of(u * T, T)
                pltpu.make_async_copy(src_k.at[b, :, pl.ds(r, T), :], kbuf.at[slot, :, pl.ds(d, T), :],
                                      ksem.at[slot]).start(priority=0)
                pltpu.make_async_copy(src_v.at[b, :, pl.ds(r, T), :], vbuf.at[slot, :, pl.ds(d, T), :],
                                      vsem.at[slot]).start(priority=1)
                return carry
            if kv_unroll:
                for k in range(n):
                    one(k, 0)
            else:
                lax.fori_loop(0, n, one, 0, unroll=unroll)

        def kv_wait(slot):
            pltpu.make_async_copy(kbuf.at[slot], kbuf.at[slot], ksem.at[slot]).wait()
            pltpu.make_async_copy(vbuf.at[slot], vbuf.at[slot], vsem.at[slot]).wait()

        def w_issue(kind, p0, n):
            def one(k, carry):
                p = p0 + k
                r = pl.multiple_of((p // NWC) * T, T)
                c = pl.multiple_of((p % NWC) * WC, WC)
                for br in range(2):
                    m = kind * 2 + br
                    pltpu.make_async_copy(w_src[m].at[:, pl.ds(r, T), pl.ds(c, WC)],
                                          w_buf.at[m, :, pl.ds(r, T), pl.ds(c, WC)],
                                          wsem.at[m * NSEG + p // SEGP]).start(priority=br)
                return carry
            lax.fori_loop(0, n, one, 0, unroll=unroll)

        def w_wait(m, seg):
            v = w_buf.at[m, :, pl.ds(pl.multiple_of(seg * SEGR, SEGR), SEGR), :]
            pltpu.make_async_copy(v, v, wsem.at[m * NSEG + seg]).wait()

        def w_load(m, seg, n=1):
            blk = w_buf[m, :, pl.ds(pl.multiple_of(seg * SEGR, SEGR), n * SEGR), :]
            return blk.reshape(WG * n * SEGR, NQ)

        row = lax.broadcasted_iota(jnp.int32, (8, DH), 0)
        rowd = lax.broadcasted_iota(jnp.int32, (8, D), 0)

        cx = [pltpu.make_async_copy(xa, x_buf.at[0], xsem.at[0]),
              pltpu.make_async_copy(xb, x_buf.at[1], xsem.at[1])]
        w_issue(0, 0, 4)
        cx[0].start(); cx[1].start()
        w_issue(0, 4, LEAD - 4)

        lhs_scr[...] = jnp.zeros(lhs_scr.shape, lhs_scr.dtype)
        z_scr[...] = jnp.zeros(z_scr.shape, z_scr.dtype)
        cx[0].wait(); cx[1].wait()
        for br in range(2):
            xv = x_buf[br].astype(jnp.float32)
            x8 = jnp.where(rowd < 2, xv[0:1], jnp.where(rowd < 4, xv[1:2], 0.0))
            for seg in range(NSEG):
                xk_scr[br * NSEG + seg] = jnp.concatenate(
                    [x8[:, g * WR + seg * SEGR:g * WR + (seg + 1) * SEGR] for g in range(WG)],
                    axis=1).astype(jnp.bfloat16)

        QI = NWP // (2 * NSEG)

        def qbody(it, carry):
            seg = it // 2
            br = it % 2
            w_wait(br, seg)
            p = LEAD + it * QI

            @pl.when(p < NWP)
            def _():
                w_issue(0, jnp.minimum(p, NWP - QI), QI)

            @pl.when(p >= NWP)
            def _():
                u = jnp.maximum(p - NWP, 0)
                s = u // U
                kv_issue(ka, va, 0, s * R, s, u - s * U, QI, kv_unroll=False)

            z_scr[br] += jnp.dot(xk_scr[br * NSEG + seg], w_load(br, seg), preferred_element_type=jnp.float32)
            return carry

        with scope("qloop"):
            lax.fori_loop(0, 2 * NSEG, qbody, 0)

        def qfin(n, carry):
            br = n // HKV
            j = n % HKV
            z = z_scr[br, :, pl.ds(pl.multiple_of(j * GW, GW), GW)]
            qj = jnp.where(row % 2 == 0, z[:, :DH], z[:, DH:])
            qj = qj.astype(jnp.bfloat16).astype(jnp.float32) * (DH ** -0.5)
            q_scr[n] = qj.astype(jnp.bfloat16)
            return carry
        lax.fori_loop(0, 2 * HKV, qfin, 0)

        def body(s, carry):
            slot = s % NBUF
            is_a = s < NA
            t = jnp.where(is_a, s, s - NA)
            b = jnp.where(is_a, t // CA, t // CB)
            cn = jnp.where(is_a, CA, CB)
            c = t - b * cn
            br = jnp.where(is_a, 0, 1)

            g = s + LEADG
            gslot = g % NBUF
            ga = jnp.minimum(g, NA - 1)
            gb = jnp.clip(g - NA, 0, NB - 1)
            gw = jnp.maximum(g - NS, 0)

            def issue_part(u0, n):
                @pl.when(g < NA)
                def _():
                    kv_issue(ka, va, ga // CA, (ga % CA) * R, gslot, u0, n)

                @pl.when(jnp.logical_and(g >= NA, g < NS))
                def _():
                    kv_issue(kb, vb, gb // CB, SK - W + (gb % CB) * R, gslot, u0, n)

                @pl.when(g >= NS)
                def _():
                    w_issue(1, gw * U + u0, n)

            kv_wait(slot)

            @pl.when(c == 0)
            def _():
                m_scr[...] = jnp.full(m_scr.shape, -jnp.inf, jnp.float32)
                l_scr[...] = jnp.zeros(l_scr.shape, jnp.float32)
                acc_scr[...] = jnp.zeros(acc_scr.shape, jnp.float32)

            hp = HKV // ISPLIT
            for part in range(ISPLIT):
                issue_part(part * U // ISPLIT, U // ISPLIT)
                for j in range(part * hp, (part + 1) * hp):
                    q = q_scr[br * HKV + j]
                    sc = lax.dot_general(q, kbuf[slot, j], _NT, preferred_element_type=jnp.float32)
                    m_prev = m_scr[j]
                    m_new = jnp.maximum(m_prev, jnp.max(sc, axis=1, keepdims=True))
                    alpha = jnp.exp(m_prev - m_new)
                    p = jnp.exp(sc - jnp.concatenate([m_new] * (R // 128), axis=1))
                    psum = p[:, 0:128]
                    for i in range(1, R // 128):
                        psum = psum + p[:, i * 128:(i + 1) * 128]
                    m_scr[j] = m_new
                    l_scr[j] = alpha * l_scr[j] + psum
                    pv = jnp.dot(p.astype(jnp.bfloat16), vbuf[slot, j], preferred_element_type=jnp.float32)
                    acc_scr[j] = jnp.concatenate([alpha] * (DH // 128), axis=1) * acc_scr[j] + pv

            @pl.when(c == cn - 1)
            def _():
                for j in range(HKV):
                    o = acc_scr[j] / jnp.sum(l_scr[j], axis=1, keepdims=True)
                    old = lhs_scr[br, :, j * GW:(j + 1) * GW].astype(jnp.float32)
                    new = jnp.concatenate(
                        [jnp.where(row == 2 * b, o, old[:, :DH]),
                         jnp.where(row == 2 * b + 1, o, old[:, DH:])], axis=1)
                    lhs_scr[br, :, j * GW:(j + 1) * GW] = new.astype(jnp.bfloat16)
            return carry

        with scope("kvloop"):
            lax.fori_loop(0, NS, body, 0)

        def store_seg(br, seg):
            y = y_scr[br * NSEG + seg]
            res = jnp.concatenate([y[0:1] + y[1:2], y[2:3] + y[3:4]], axis=0).astype(out_ref.dtype)
            for g in range(WG):
                o0 = br * D + g * WR + seg * SEGR
                out_ref[:, o0:o0 + SEGR] = res[:, g * SEGR:(g + 1) * SEGR]

        def sel(it, vals):
            out = jnp.int32(vals[0])
            for k in range(1, len(vals)):
                out = jnp.where(it >= k, jnp.int32(vals[k]), out)
            return out

        n_oi = (NWP - LEAD) // OI
        for it, (br, seg) in enumerate(o_sched):
            assert (seg + 1) * SEGP <= LEAD + min(it, n_oi) * OI, (it, br, seg)

        def obody(it, carry):
            br = sel(it, [x[0] for x in o_sched])
            seg = sel(it, [x[1] for x in o_sched])
            with scope("ow"):
                w_wait(2 + br, seg)

            @pl.when(it < n_oi)
            def _():
                w_issue(1, LEAD + jnp.minimum(it, n_oi - 1) * OI, OI)

            with scope("oc"):
                y_scr[br * NSEG + seg] = lax.dot_general(lhs_scr[br], w_load(2 + br, seg), _NT,
                                                         preferred_element_type=jnp.float32)

            @pl.when(it == 2 * NSEG - asm_at)
            def _():
                for (b2, s2) in o_sched[:2 * NSEG - asm_at + 1]:
                    store_seg(b2, s2)
            return carry

        with scope("oloop"):
            lax.fori_loop(0, 2 * NSEG, obody, 0)
        for (b2, s2) in o_sched[2 * NSEG - asm_at + 1:]:
            store_seg(b2, s2)

    @jax.jit
    def fn(A_x, A_k_cache, A_v_cache, A_wq, A_wo, B_x, B_k_cache, B_v_cache, B_wq, B_wo):
        def prep(x, k, v, wq, wo):
            return (x.reshape(B, D), k, v, wq.reshape(WG, WR, NQ), wo.T.reshape(WG, WR, NQ))
        bf16, f32 = jnp.bfloat16, jnp.float32
        out = pl.pallas_call(
            kernel,
            out_shape=jax.ShapeDtypeStruct((B, 2 * D), bf16),
            in_specs=[pl.BlockSpec(memory_space=pltpu.HBM)] * 10,
            out_specs=pl.BlockSpec(memory_space=pltpu.VMEM),
            scratch_shapes=[
                pltpu.VMEM((NBUF, HKV, R, DH), bf16),
                pltpu.VMEM((NBUF, HKV, R, DH), bf16),
                pltpu.VMEM((4, WG, WR, NQ), bf16),
                pltpu.VMEM((2, B, D), bf16),
                pltpu.VMEM((2 * NSEG, 8, WG * SEGR), bf16),
                pltpu.VMEM((2 * HKV, 8, DH), bf16),
                pltpu.VMEM((2, 8, NQ), f32),
                pltpu.VMEM((HKV, 8, 128), f32),
                pltpu.VMEM((HKV, 8, 128), f32),
                pltpu.VMEM((HKV, 8, DH), f32),
                pltpu.VMEM((2, 8, NQ), bf16),
                pltpu.VMEM((2 * NSEG, 8, WG * SEGR), f32),
                pltpu.SemaphoreType.DMA((NBUF,)),
                pltpu.SemaphoreType.DMA((NBUF,)),
                pltpu.SemaphoreType.DMA((4 * NSEG,)),
                pltpu.SemaphoreType.DMA((2,)),
            ],
            compiler_params=pltpu.CompilerParams(
                vmem_limit_bytes=64 * 1024 * 1024,
                disable_bounds_checks=nobc,
                disable_semaphore_checks=nosc,
            ),
        )(*prep(A_x, A_k_cache, A_v_cache, A_wq, A_wo),
          *prep(B_x, B_k_cache, B_v_cache, B_wq, B_wo))
        return out.reshape(B, 1, 2 * D)
    return fn


pallas_concat_heads__gqa_block_cached__sliding_block_cached__decode_kernel = make(**dict())
```

```python
import jax
import jax.numpy as jnp
from jax import lax
import jax.experimental.pallas as pl
import jax.experimental.pallas.tpu as pltpu

B, D = 2, 448
HQ, HKV, SK, DH = 16, 8, 8192, 256
REP = HQ // HKV
W = min(4096, max(256, SK // 4))
GW = REP * DH
NQ = HQ * DH

T = 8
R = 256
U = R // T
NBUF = 3
LEADG = NBUF - 1
LEAD = LEADG * U
CA, CB = SK // R, W // R
NA, NB = B * CA, B * CB
NS = NA + NB
ISPLIT = 2

WG, WR, WC = 4, 112, 512
NWC = NQ // WC
NWP = (WR // T) * NWC
SEGR = 16
NSEG = WR // SEGR
SEGP = (SEGR // T) * NWC
QI = NWP // (2 * NSEG)
OI = 8
N_OI = (NWP - LEAD) // OI
O_SCHED = ((0, 0), (0, 1), (1, 0), (0, 2), (1, 1), (0, 3), (1, 2),
           (0, 4), (1, 3), (0, 5), (1, 4), (0, 6), (1, 5), (1, 6))
for _it, (_br, _seg) in enumerate(O_SCHED):
    assert (_seg + 1) * SEGP <= LEAD + min(_it, N_OI) * OI

_NT = (((1,), (1,)), ((), ()))


def _kernel(xa, ka, va, wqa, woa, xb, kb, vb, wqb, wob, out_ref,
            kbuf, vbuf, w_buf, x_buf, xk_scr, q_scr, z_scr, m_scr, l_scr, acc_scr,
            lhs_scr, y_scr, ksem, vsem, wsem, xsem):
    w_src = (wqa, wqb, woa, wob)

    def kv_issue(src_k, src_v, b, row0, slot, u0, n):
        for k in range(n):
            r = pl.multiple_of(row0 + (u0 + k) * T, T)
            d = pl.multiple_of((u0 + k) * T, T)
            pltpu.make_async_copy(src_k.at[b, :, pl.ds(r, T), :],
                                  kbuf.at[slot, :, pl.ds(d, T), :],
                                  ksem.at[slot]).start(priority=0)
            pltpu.make_async_copy(src_v.at[b, :, pl.ds(r, T), :],
                                  vbuf.at[slot, :, pl.ds(d, T), :],
                                  vsem.at[slot]).start(priority=1)

    def kv_wait(slot):
        pltpu.make_async_copy(kbuf.at[slot], kbuf.at[slot], ksem.at[slot]).wait()
        pltpu.make_async_copy(vbuf.at[slot], vbuf.at[slot], vsem.at[slot]).wait()

    def w_issue(kind, p0, n):
        def one(k, carry):
            p = p0 + k
            r = pl.multiple_of((p // NWC) * T, T)
            c = pl.multiple_of((p % NWC) * WC, WC)
            for br in range(2):
                m = kind * 2 + br
                pltpu.make_async_copy(w_src[m].at[:, pl.ds(r, T), pl.ds(c, WC)],
                                      w_buf.at[m, :, pl.ds(r, T), pl.ds(c, WC)],
                                      wsem.at[m * NSEG + p // SEGP]).start(priority=br)
            return carry
        lax.fori_loop(0, n, one, 0, unroll=4)

    def w_wait(m, seg):
        v = w_buf.at[m, :, pl.ds(pl.multiple_of(seg * SEGR, SEGR), SEGR), :]
        pltpu.make_async_copy(v, v, wsem.at[m * NSEG + seg]).wait()

    def w_load(m, seg):
        blk = w_buf[m, :, pl.ds(pl.multiple_of(seg * SEGR, SEGR), SEGR), :]
        return blk.reshape(WG * SEGR, NQ)

    row = lax.broadcasted_iota(jnp.int32, (8, DH), 0)
    rowd = lax.broadcasted_iota(jnp.int32, (8, D), 0)

    cx = [pltpu.make_async_copy(xa, x_buf.at[0], xsem.at[0]),
          pltpu.make_async_copy(xb, x_buf.at[1], xsem.at[1])]
    w_issue(0, 0, 4)
    cx[0].start()
    cx[1].start()
    w_issue(0, 4, LEAD - 4)

    lhs_scr[...] = jnp.zeros(lhs_scr.shape, lhs_scr.dtype)
    z_scr[...] = jnp.zeros(z_scr.shape, z_scr.dtype)
    cx[0].wait()
    cx[1].wait()
    for br in range(2):
        xv = x_buf[br].astype(jnp.float32)
        x8 = jnp.where(rowd < 2, xv[0:1], jnp.where(rowd < 4, xv[1:2], 0.0))
        for seg in range(NSEG):
            xk = [x8[:, g * WR + seg * SEGR:g * WR + (seg + 1) * SEGR] for g in range(WG)]
            xk_scr[br * NSEG + seg] = jnp.concatenate(xk, axis=1).astype(jnp.bfloat16)

    def q_step(it, carry):
        seg = it // 2
        br = it % 2
        w_wait(br, seg)
        p = LEAD + it * QI

        @pl.when(p < NWP)
        def _():
            w_issue(0, jnp.minimum(p, NWP - QI), QI)

        @pl.when(p >= NWP)
        def _():
            u = jnp.maximum(p - NWP, 0)
            s = u // U
            kv_issue(ka, va, 0, s * R, s, u - s * U, QI)

        z_scr[br] += jnp.dot(xk_scr[br * NSEG + seg], w_load(br, seg),
                             preferred_element_type=jnp.float32)
        return carry

    lax.fori_loop(0, 2 * NSEG, q_step, 0)

    def q_final(n, carry):
        z = z_scr[n // HKV, :, pl.ds(pl.multiple_of((n % HKV) * GW, GW), GW)]
        q = jnp.where(row % 2 == 0, z[:, :DH], z[:, DH:])
        q = q.astype(jnp.bfloat16).astype(jnp.float32) * (DH ** -0.5)
        q_scr[n] = q.astype(jnp.bfloat16)
        return carry

    lax.fori_loop(0, 2 * HKV, q_final, 0)

    def kv_step(s, carry):
        slot = s % NBUF
        is_a = s < NA
        t = jnp.where(is_a, s, s - NA)
        b = jnp.where(is_a, t // CA, t // CB)
        cn = jnp.where(is_a, CA, CB)
        c = t - b * cn
        br = jnp.where(is_a, 0, 1)

        g = s + LEADG
        gslot = g % NBUF
        ga = jnp.minimum(g, NA - 1)
        gb = jnp.clip(g - NA, 0, NB - 1)
        gw = jnp.maximum(g - NS, 0)

        def issue_part(u0, n):
            @pl.when(g < NA)
            def _():
                kv_issue(ka, va, ga // CA, (ga % CA) * R, gslot, u0, n)

            @pl.when(jnp.logical_and(g >= NA, g < NS))
            def _():
                kv_issue(kb, vb, gb // CB, SK - W + (gb % CB) * R, gslot, u0, n)

            @pl.when(g >= NS)
            def _():
                w_issue(1, gw * U + u0, n)

        kv_wait(slot)

        @pl.when(c == 0)
        def _():
            m_scr[...] = jnp.full(m_scr.shape, -jnp.inf, jnp.float32)
            l_scr[...] = jnp.zeros(l_scr.shape, jnp.float32)
            acc_scr[...] = jnp.zeros(acc_scr.shape, jnp.float32)

        hp = HKV // ISPLIT
        for part in range(ISPLIT):
            issue_part(part * U // ISPLIT, U // ISPLIT)
            for j in range(part * hp, (part + 1) * hp):
                sc = lax.dot_general(q_scr[br * HKV + j], kbuf[slot, j], _NT,
                                     preferred_element_type=jnp.float32)
                m_prev = m_scr[j]
                m_new = jnp.maximum(m_prev, jnp.max(sc, axis=1, keepdims=True))
                alpha = jnp.exp(m_prev - m_new)
                p = jnp.exp(sc - jnp.concatenate([m_new] * (R // 128), axis=1))
                psum = p[:, 0:128]
                for i in range(1, R // 128):
                    psum = psum + p[:, i * 128:(i + 1) * 128]
                m_scr[j] = m_new
                l_scr[j] = alpha * l_scr[j] + psum
                pv = jnp.dot(p.astype(jnp.bfloat16), vbuf[slot, j],
                             preferred_element_type=jnp.float32)
                acc_scr[j] = jnp.concatenate([alpha] * (DH // 128), axis=1) * acc_scr[j] + pv

        @pl.when(c == cn - 1)
        def _():
            for j in range(HKV):
                o = acc_scr[j] / jnp.sum(l_scr[j], axis=1, keepdims=True)
                old = lhs_scr[br, :, j * GW:(j + 1) * GW].astype(jnp.float32)
                new = jnp.concatenate(
                    [jnp.where(row == 2 * b, o, old[:, :DH]),
                     jnp.where(row == 2 * b + 1, o, old[:, DH:])], axis=1)
                lhs_scr[br, :, j * GW:(j + 1) * GW] = new.astype(jnp.bfloat16)

        return carry

    lax.fori_loop(0, NS, kv_step, 0)

    def emit(br, seg):
        y = y_scr[br * NSEG + seg]
        res = jnp.concatenate([y[0:1] + y[1:2], y[2:3] + y[3:4]], axis=0)
        res = res.astype(out_ref.dtype)
        for g in range(WG):
            o0 = br * D + g * WR + seg * SEGR
            out_ref[:, o0:o0 + SEGR] = res[:, g * SEGR:(g + 1) * SEGR]

    def pick(it, vals):
        out = jnp.int32(vals[0])
        for k in range(1, len(vals)):
            out = jnp.where(it >= k, jnp.int32(vals[k]), out)
        return out

    def o_step(it, carry):
        br = pick(it, [e[0] for e in O_SCHED])
        seg = pick(it, [e[1] for e in O_SCHED])
        w_wait(2 + br, seg)

        @pl.when(it < N_OI)
        def _():
            w_issue(1, LEAD + jnp.minimum(it, N_OI - 1) * OI, OI)

        y_scr[br * NSEG + seg] = lax.dot_general(lhs_scr[br], w_load(2 + br, seg), _NT,
                                                 preferred_element_type=jnp.float32)

        @pl.when(it == len(O_SCHED) - 2)
        def _():
            for e in O_SCHED[:-1]:
                emit(*e)

        return carry

    lax.fori_loop(0, len(O_SCHED), o_step, 0)
    emit(*O_SCHED[-1])


@jax.jit
def pallas_concat_heads__gqa_block_cached__sliding_block_cached__decode_kernel(
    A_x: jax.Array,
    A_k_cache: jax.Array,
    A_v_cache: jax.Array,
    A_wq: jax.Array,
    A_wo: jax.Array,
    B_x: jax.Array,
    B_k_cache: jax.Array,
    B_v_cache: jax.Array,
    B_wq: jax.Array,
    B_wo: jax.Array,
):
    assert A_x.shape == B_x.shape == (B, 1, D)
    assert A_k_cache.shape == A_v_cache.shape == (B, HKV, SK, DH)
    assert B_k_cache.shape == B_v_cache.shape == (B, HKV, SK, DH)
    assert A_wq.shape == B_wq.shape == (D, NQ)
    assert A_wo.shape == B_wo.shape == (NQ, D)

    def prep(x, k, v, wq, wo):
        return (x.reshape(B, D), k, v, wq.reshape(WG, WR, NQ), wo.T.reshape(WG, WR, NQ))

    bf16, f32 = jnp.bfloat16, jnp.float32
    out = pl.pallas_call(
        _kernel,
        out_shape=jax.ShapeDtypeStruct((B, 2 * D), bf16),
        in_specs=[pl.BlockSpec(memory_space=pltpu.HBM)] * 10,
        out_specs=pl.BlockSpec(memory_space=pltpu.VMEM),
        scratch_shapes=[
            pltpu.VMEM((NBUF, HKV, R, DH), bf16),
            pltpu.VMEM((NBUF, HKV, R, DH), bf16),
            pltpu.VMEM((4, WG, WR, NQ), bf16),
            pltpu.VMEM((2, B, D), bf16),
            pltpu.VMEM((2 * NSEG, 8, WG * SEGR), bf16),
            pltpu.VMEM((2 * HKV, 8, DH), bf16),
            pltpu.VMEM((2, 8, NQ), f32),
            pltpu.VMEM((HKV, 8, 128), f32),
            pltpu.VMEM((HKV, 8, 128), f32),
            pltpu.VMEM((HKV, 8, DH), f32),
            pltpu.VMEM((2, 8, NQ), bf16),
            pltpu.VMEM((2 * NSEG, 8, WG * SEGR), f32),
            pltpu.SemaphoreType.DMA((NBUF,)),
            pltpu.SemaphoreType.DMA((NBUF,)),
            pltpu.SemaphoreType.DMA((4 * NSEG,)),
            pltpu.SemaphoreType.DMA((2,)),
        ],
        compiler_params=pltpu.CompilerParams(
            vmem_limit_bytes=64 * 1024 * 1024,
            disable_bounds_checks=True,
            disable_semaphore_checks=True,
        ),
    )(*prep(A_x, A_k_cache, A_v_cache, A_wq, A_wo),
      *prep(B_x, B_k_cache, B_v_cache, B_wq, B_wo))
    return out.reshape(B, 1, 2 * D)
```

```python
import jax
import jax.numpy as jnp
from jax import lax
import jax.experimental.pallas as pl
import jax.experimental.pallas.tpu as pltpu

B, D = 2, 448
HQ, HKV, SK, DH = 16, 8, 8192, 256
REP = HQ // HKV
W = min(4096, max(256, SK // 4))
GW = REP * DH
NQ = HQ * DH

T = 8
R = 256
U = R // T
NBUF = 3
LEADG = NBUF - 1
LEAD = LEADG * U
CA, CB = SK // R, W // R
NA, NB = B * CA, B * CB
NS = NA + NB
ISPLIT = 2

WG, WR, WC = 4, 112, 512
NWC = NQ // WC
NWP = (WR // T) * NWC
SEGR = 16
NSEG = WR // SEGR
SEGP = (SEGR // T) * NWC
QI = NWP // (2 * NSEG)
OI = 8
N_OI = (NWP - SEGP - LEAD) // OI
NP = 2
ASMB = 2
O_SCHED = ((0, 0), (0, 1), (1, 0), (0, 2), (1, 1), (0, 3), (1, 2),
           (0, 4), (1, 3), (0, 5), (1, 4), (0, 6), (1, 5), (1, 6))
for _it, (_br, _seg) in enumerate(O_SCHED):
    assert (_seg + 1) * SEGP <= LEAD + min(_it, N_OI) * OI + (SEGP if _it > N_OI else 0)

_NT = (((1,), (1,)), ((), ()))


def _kernel(xa, ka, va, wqa, woa, xb, kb, vb, wqb, wob, out_ref,
            kbuf, vbuf, w_buf, x_buf, xk_scr, q_scr, z_scr, m_scr, l_scr, acc_scr,
            lhs_scr, y_scr, ksem, vsem, wsem, xsem):
    w_src = (wqa, wqb, woa, wob)

    def kv_issue(src_k, src_v, b, row0, slot, u0, n):
        for k in range(n):
            r = pl.multiple_of(row0 + (u0 + k) * T, T)
            d = pl.multiple_of((u0 + k) * T, T)
            pltpu.make_async_copy(src_k.at[b, :, pl.ds(r, T), :],
                                  kbuf.at[slot, :, pl.ds(d, T), :],
                                  ksem.at[slot]).start(priority=0)
            pltpu.make_async_copy(src_v.at[b, :, pl.ds(r, T), :],
                                  vbuf.at[slot, :, pl.ds(d, T), :],
                                  vsem.at[slot]).start(priority=1)

    def kv_wait(slot):
        pltpu.make_async_copy(kbuf.at[slot], kbuf.at[slot], ksem.at[slot]).wait()
        pltpu.make_async_copy(vbuf.at[slot], vbuf.at[slot], vsem.at[slot]).wait()

    def w_issue(kind, p0, n):
        def one(k, carry):
            p = p0 + k
            r = pl.multiple_of((p // NWC) * T, T)
            c = pl.multiple_of((p % NWC) * WC, WC)
            for br in range(2):
                m = kind * 2 + br
                pltpu.make_async_copy(w_src[m].at[:, pl.ds(r, T), pl.ds(c, WC)],
                                      w_buf.at[m, :, pl.ds(r, T), pl.ds(c, WC)],
                                      wsem.at[m * NSEG + p // SEGP]).start(priority=br)
            return carry
        lax.fori_loop(0, n, one, 0, unroll=4)

    def w_wait(m, seg):
        v = w_buf.at[m, :, pl.ds(pl.multiple_of(seg * SEGR, SEGR), SEGR), :]
        pltpu.make_async_copy(v, v, wsem.at[m * NSEG + seg]).wait()

    def w_load(m, seg):
        blk = w_buf[m, :, pl.ds(pl.multiple_of(seg * SEGR, SEGR), SEGR), :]
        return blk.reshape(WG * SEGR, NQ)

    row = lax.broadcasted_iota(jnp.int32, (8, DH), 0)
    rowd = lax.broadcasted_iota(jnp.int32, (8, D), 0)

    cx = [pltpu.make_async_copy(xa, x_buf.at[0], xsem.at[0]),
          pltpu.make_async_copy(xb, x_buf.at[1], xsem.at[1])]
    w_issue(0, 0, 4)
    cx[0].start()
    cx[1].start()
    w_issue(0, 4, LEAD - 4)

    lhs_scr[...] = jnp.zeros(lhs_scr.shape, lhs_scr.dtype)
    z_scr[...] = jnp.zeros(z_scr.shape, z_scr.dtype)
    cx[0].wait()
    cx[1].wait()
    for br in range(2):
        xv = x_buf[br].astype(jnp.float32)
        x8 = jnp.where(rowd < 2, xv[0:1], jnp.where(rowd < 4, xv[1:2], 0.0))
        for seg in range(NSEG):
            xk = [x8[:, g * WR + seg * SEGR:g * WR + (seg + 1) * SEGR] for g in range(WG)]
            xk_scr[br * NSEG + seg] = jnp.concatenate(xk, axis=1).astype(jnp.bfloat16)

    def q_step(it, carry):
        seg = it // 2
        br = it % 2
        w_wait(br, seg)
        p = LEAD + it * QI

        @pl.when(p < NWP)
        def _():
            w_issue(0, jnp.minimum(p, NWP - QI), QI)

        @pl.when(p >= NWP)
        def _():
            u = jnp.maximum(p - NWP, 0)
            s = u // U
            kv_issue(ka, va, 0, s * R, s, u - s * U, QI)

        z_scr[br] += jnp.dot(xk_scr[br * NSEG + seg], w_load(br, seg),
                             preferred_element_type=jnp.float32)
        return carry

    lax.fori_loop(0, 2 * NSEG, q_step, 0)

    def q_final(n, carry):
        z = z_scr[n // HKV, :, pl.ds(pl.multiple_of((n % HKV) * GW, GW), GW)]
        q = jnp.where(row % 2 == 0, z[:, :DH], z[:, DH:])
        q = q.astype(jnp.bfloat16).astype(jnp.float32) * (DH ** -0.5)
        q_scr[n] = q.astype(jnp.bfloat16)
        return carry

    lax.fori_loop(0, 2 * HKV, q_final, 0)

    def kv_step(s, carry):
        slot = s % NBUF
        is_a = s < NA
        t = jnp.where(is_a, s, s - NA)
        b = jnp.where(is_a, t // CA, t // CB)
        cn = jnp.where(is_a, CA, CB)
        c = t - b * cn
        br = jnp.where(is_a, 0, 1)

        g = s + LEADG
        gslot = g % NBUF
        ga = jnp.minimum(g, NA - 1)
        gb = jnp.clip(g - NA, 0, NB - 1)
        gw = jnp.maximum(g - NS, 0)

        def issue_part(u0, n):
            @pl.when(g < NA)
            def _():
                kv_issue(ka, va, ga // CA, (ga % CA) * R, gslot, u0, n)

            @pl.when(jnp.logical_and(g >= NA, g < NS))
            def _():
                kv_issue(kb, vb, gb // CB, SK - W + (gb % CB) * R, gslot, u0, n)

            @pl.when(g >= NS)
            def _():
                w_issue(1, gw * U + u0, n)

        kv_wait(slot)

        @pl.when(c == 0)
        def _():
            m_scr[...] = jnp.full(m_scr.shape, -jnp.inf, jnp.float32)
            l_scr[...] = jnp.zeros(l_scr.shape, jnp.float32)
            acc_scr[...] = jnp.zeros(acc_scr.shape, jnp.float32)

        hp = HKV // ISPLIT
        for part in range(ISPLIT):
            issue_part(part * U // ISPLIT, U // ISPLIT)
            for j in range(part * hp, (part + 1) * hp):
                sc = lax.dot_general(q_scr[br * HKV + j], kbuf[slot, j], _NT,
                                     preferred_element_type=jnp.float32)
                m_prev = m_scr[j]
                m_new = jnp.maximum(m_prev, jnp.max(sc, axis=1, keepdims=True))
                alpha = jnp.exp(m_prev - m_new)
                p = jnp.exp(sc - jnp.concatenate([m_new] * (R // 128), axis=1))
                psum = p[:, 0:128]
                for i in range(1, R // 128):
                    psum = psum + p[:, i * 128:(i + 1) * 128]
                m_scr[j] = m_new
                l_scr[j] = alpha * l_scr[j] + psum
                pv = jnp.dot(p.astype(jnp.bfloat16), vbuf[slot, j],
                             preferred_element_type=jnp.float32)
                acc_scr[j] = jnp.concatenate([alpha] * (DH // 128), axis=1) * acc_scr[j] + pv

        @pl.when(c == cn - 1)
        def _():
            for j in range(HKV):
                o = acc_scr[j] / jnp.sum(l_scr[j], axis=1, keepdims=True)
                old = lhs_scr[br, :, j * GW:(j + 1) * GW].astype(jnp.float32)
                new = jnp.concatenate(
                    [jnp.where(row == 2 * b, o, old[:, :DH]),
                     jnp.where(row == 2 * b + 1, o, old[:, DH:])], axis=1)
                lhs_scr[br, :, j * GW:(j + 1) * GW] = new.astype(jnp.bfloat16)

        return carry

    lax.fori_loop(0, NS, kv_step, 0)

    def emit(br, seg):
        y = y_scr[br * NSEG + seg]
        res = jnp.concatenate([y[0:1] + y[1:2], y[2:3] + y[3:4]], axis=0)
        res = res.astype(out_ref.dtype)
        for g in range(WG):
            o0 = br * D + g * WR + seg * SEGR
            out_ref[:, o0:o0 + SEGR] = res[:, g * SEGR:(g + 1) * SEGR]

    def pick(it, vals):
        out = jnp.int32(vals[0])
        for k in range(1, len(vals)):
            out = jnp.where(it >= k, jnp.int32(vals[k]), out)
        return out

    def issue_last():
        i0 = (NSEG - 1) * SEGR // T
        la = [(i, c) for i in range(i0, i0 + SEGR // T) for c in range(NWC)]
        lb = [(i, t * (NWC // NP) + c, t) for t in range(NP)
              for i in range(i0, i0 + SEGR // T) for c in range(NWC // NP)]
        for (ia, ca), (ib, cb, t) in zip(la, lb):
            pltpu.make_async_copy(woa.at[:, pl.ds(ia * T, T), pl.ds(ca * WC, WC)],
                                  w_buf.at[2, :, pl.ds(ia * T, T), pl.ds(ca * WC, WC)],
                                  wsem.at[3 * NSEG - 1]).start(priority=0)
            pltpu.make_async_copy(wob.at[:, pl.ds(ib * T, T), pl.ds(cb * WC, WC)],
                                  w_buf.at[3, :, pl.ds(ib * T, T), pl.ds(cb * WC, WC)],
                                  wsem.at[4 * NSEG - 1 + t]).start(priority=1)

    def o_step(it, carry):
        br = pick(it, [e[0] for e in O_SCHED[:-1]])
        seg = pick(it, [e[1] for e in O_SCHED[:-1]])
        w_wait(2 + br, seg)

        @pl.when(it < N_OI)
        def _():
            w_issue(1, LEAD + jnp.minimum(it, N_OI - 1) * OI, OI)

        @pl.when(it == N_OI)
        def _():
            issue_last()

        y_scr[br * NSEG + seg] = lax.dot_general(lhs_scr[br], w_load(2 + br, seg), _NT,
                                                 preferred_element_type=jnp.float32)

        @pl.when(it == len(O_SCHED) - 2 - ASMB)
        def _():
            for e in O_SCHED[:-1 - ASMB]:
                emit(*e)

        return carry

    lax.fori_loop(0, len(O_SCHED) - 1, o_step, 0)
    for e in O_SCHED[len(O_SCHED) - 1 - ASMB:-1]:
        emit(*e)

    KP = NQ // NP
    r0 = (NSEG - 1) * SEGR

    def t_step(t, y):
        k0 = pl.multiple_of(t * KP, KP)
        v = w_buf.at[3, :, pl.ds(r0, SEGR), pl.ds(k0, KP)]
        pltpu.make_async_copy(v, v, wsem.at[4 * NSEG - 1 + t]).wait()
        blk = w_buf[3, :, pl.ds(r0, SEGR), pl.ds(k0, KP)].reshape(WG * SEGR, KP)
        return y + lax.dot_general(lhs_scr[1, :, pl.ds(k0, KP)], blk, _NT,
                                   preferred_element_type=jnp.float32)

    y_scr[2 * NSEG - 1] = lax.fori_loop(0, NP, t_step, jnp.zeros((8, WG * SEGR), jnp.float32))
    emit(*O_SCHED[-1])


@jax.jit
def pallas_concat_heads__gqa_block_cached__sliding_block_cached__decode_kernel(
    A_x: jax.Array,
    A_k_cache: jax.Array,
    A_v_cache: jax.Array,
    A_wq: jax.Array,
    A_wo: jax.Array,
    B_x: jax.Array,
    B_k_cache: jax.Array,
    B_v_cache: jax.Array,
    B_wq: jax.Array,
    B_wo: jax.Array,
):
    assert A_x.shape == B_x.shape == (B, 1, D)
    assert A_k_cache.shape == A_v_cache.shape == (B, HKV, SK, DH)
    assert B_k_cache.shape == B_v_cache.shape == (B, HKV, SK, DH)
    assert A_wq.shape == B_wq.shape == (D, NQ)
    assert A_wo.shape == B_wo.shape == (NQ, D)

    def prep(x, k, v, wq, wo):
        return (x.reshape(B, D), k, v, wq.reshape(WG, WR, NQ), wo.T.reshape(WG, WR, NQ))

    bf16, f32 = jnp.bfloat16, jnp.float32
    out = pl.pallas_call(
        _kernel,
        out_shape=jax.ShapeDtypeStruct((B, 2 * D), bf16),
        in_specs=[pl.BlockSpec(memory_space=pltpu.HBM)] * 10,
        out_specs=pl.BlockSpec(memory_space=pltpu.VMEM),
        scratch_shapes=[
            pltpu.VMEM((NBUF, HKV, R, DH), bf16),
            pltpu.VMEM((NBUF, HKV, R, DH), bf16),
            pltpu.VMEM((4, WG, WR, NQ), bf16),
            pltpu.VMEM((2, B, D), bf16),
            pltpu.VMEM((2 * NSEG, 8, WG * SEGR), bf16),
            pltpu.VMEM((2 * HKV, 8, DH), bf16),
            pltpu.VMEM((2, 8, NQ), f32),
            pltpu.VMEM((HKV, 8, 128), f32),
            pltpu.VMEM((HKV, 8, 128), f32),
            pltpu.VMEM((HKV, 8, DH), f32),
            pltpu.VMEM((2, 8, NQ), bf16),
            pltpu.VMEM((2 * NSEG, 8, WG * SEGR), f32),
            pltpu.SemaphoreType.DMA((NBUF,)),
            pltpu.SemaphoreType.DMA((NBUF,)),
            pltpu.SemaphoreType.DMA((4 * NSEG - 1 + NP,)),
            pltpu.SemaphoreType.DMA((2,)),
        ],
        compiler_params=pltpu.CompilerParams(
            vmem_limit_bytes=64 * 1024 * 1024,
            disable_bounds_checks=True,
            disable_semaphore_checks=True,
        ),
    )(*prep(A_x, A_k_cache, A_v_cache, A_wq, A_wo),
      *prep(B_x, B_k_cache, B_v_cache, B_wq, B_wo))
    return out.reshape(B, 1, 2 * D)
```

```python
import jax
import jax.numpy as jnp
from jax import lax
import jax.experimental.pallas as pl
import jax.experimental.pallas.tpu as pltpu

B, D = 2, 448
HQ, HKV, SK, DH = 16, 8, 8192, 256
REP = HQ // HKV
W = min(4096, max(256, SK // 4))
GW = REP * DH
NQ = HQ * DH

T = 8
R = 256
U = R // T
NBUF = 3
LEADG = NBUF - 1
LEAD = LEADG * U
CA, CB = SK // R, W // R
NA, NB = B * CA, B * CB
NS = NA + NB
ISPLIT = 2

WG, WR, WC = 4, 112, 512
NWC = NQ // WC
NWP = (WR // T) * NWC
SEGR = 16
NSEG = WR // SEGR
SEGP = (SEGR // T) * NWC
QI = NWP // (2 * NSEG)
OI = 8
N_OI = (NWP - SEGP - LEAD) // OI
NP = 2
N_LATE = 2
O_SCHED = ((0, 0), (0, 1), (1, 0), (0, 2), (1, 1), (0, 3), (1, 2),
           (0, 4), (1, 3), (0, 5), (1, 4), (0, 6), (1, 5), (1, 6))
assert O_SCHED[-1] == (1, NSEG - 1)
for _it, (_br, _seg) in enumerate(O_SCHED):
    assert (_seg + 1) * SEGP <= LEAD + min(_it, N_OI) * OI + (SEGP if _it > N_OI else 0)

_NT = (((1,), (1,)), ((), ()))


def _kernel(xa, ka, va, wqa, woa, xb, kb, vb, wqb, wob, out_ref,
            kbuf, vbuf, w_buf, x_buf, xk_scr, q_scr, z_scr, m_scr, l_scr, acc_scr,
            lhs_scr, y_scr, ksem, vsem, wsem, xsem):
    w_src = (wqa, wqb, woa, wob)

    def kv_issue(src_k, src_v, b, row0, slot, u0, n):
        for k in range(n):
            r = pl.multiple_of(row0 + (u0 + k) * T, T)
            d = pl.multiple_of((u0 + k) * T, T)
            pltpu.make_async_copy(src_k.at[b, :, pl.ds(r, T), :],
                                  kbuf.at[slot, :, pl.ds(d, T), :],
                                  ksem.at[slot]).start(priority=0)
            pltpu.make_async_copy(src_v.at[b, :, pl.ds(r, T), :],
                                  vbuf.at[slot, :, pl.ds(d, T), :],
                                  vsem.at[slot]).start(priority=1)

    def kv_wait(slot):
        pltpu.make_async_copy(kbuf.at[slot], kbuf.at[slot], ksem.at[slot]).wait()
        pltpu.make_async_copy(vbuf.at[slot], vbuf.at[slot], vsem.at[slot]).wait()

    def w_issue(kind, p0, n):
        def one(k, carry):
            p = p0 + k
            r = pl.multiple_of((p // NWC) * T, T)
            c = pl.multiple_of((p % NWC) * WC, WC)
            for br in range(2):
                m = kind * 2 + br
                pltpu.make_async_copy(w_src[m].at[:, pl.ds(r, T), pl.ds(c, WC)],
                                      w_buf.at[m, :, pl.ds(r, T), pl.ds(c, WC)],
                                      wsem.at[m * NSEG + p // SEGP]).start(priority=br)
            return carry
        lax.fori_loop(0, n, one, 0, unroll=4)

    def w_wait(m, seg):
        v = w_buf.at[m, :, pl.ds(pl.multiple_of(seg * SEGR, SEGR), SEGR), :]
        pltpu.make_async_copy(v, v, wsem.at[m * NSEG + seg]).wait()

    def w_load(m, seg):
        blk = w_buf[m, :, pl.ds(pl.multiple_of(seg * SEGR, SEGR), SEGR), :]
        return blk.reshape(WG * SEGR, NQ)

    row = lax.broadcasted_iota(jnp.int32, (8, DH), 0)
    rowd = lax.broadcasted_iota(jnp.int32, (8, D), 0)

    cx = [pltpu.make_async_copy(xa, x_buf.at[0], xsem.at[0]),
          pltpu.make_async_copy(xb, x_buf.at[1], xsem.at[1])]
    w_issue(0, 0, 4)
    cx[0].start()
    cx[1].start()
    w_issue(0, 4, LEAD - 4)

    lhs_scr[...] = jnp.zeros(lhs_scr.shape, lhs_scr.dtype)
    z_scr[...] = jnp.zeros(z_scr.shape, z_scr.dtype)
    cx[0].wait()
    cx[1].wait()
    for br in range(2):
        xv = x_buf[br].astype(jnp.float32)
        x8 = jnp.where(rowd < 2, xv[0:1], jnp.where(rowd < 4, xv[1:2], 0.0))
        for seg in range(NSEG):
            xk = [x8[:, g * WR + seg * SEGR:g * WR + (seg + 1) * SEGR] for g in range(WG)]
            xk_scr[br * NSEG + seg] = jnp.concatenate(xk, axis=1).astype(jnp.bfloat16)

    def q_step(it, carry):
        seg = it // 2
        br = it % 2
        w_wait(br, seg)
        p = LEAD + it * QI

        @pl.when(p < NWP)
        def _():
            w_issue(0, jnp.minimum(p, NWP - QI), QI)

        @pl.when(p >= NWP)
        def _():
            u = jnp.maximum(p - NWP, 0)
            s = u // U
            kv_issue(ka, va, 0, s * R, s, u - s * U, QI)

        z_scr[br] += jnp.dot(xk_scr[br * NSEG + seg], w_load(br, seg),
                             preferred_element_type=jnp.float32)
        return carry

    lax.fori_loop(0, 2 * NSEG, q_step, 0)

    def q_final(n, carry):
        z = z_scr[n // HKV, :, pl.ds(pl.multiple_of((n % HKV) * GW, GW), GW)]
        q = jnp.where(row % 2 == 0, z[:, :DH], z[:, DH:])
        q = q.astype(jnp.bfloat16).astype(jnp.float32) * (DH ** -0.5)
        q_scr[n] = q.astype(jnp.bfloat16)
        return carry

    lax.fori_loop(0, 2 * HKV, q_final, 0)

    def kv_step(s, carry):
        slot = s % NBUF
        is_a = s < NA
        t = jnp.where(is_a, s, s - NA)
        b = jnp.where(is_a, t // CA, t // CB)
        cn = jnp.where(is_a, CA, CB)
        c = t - b * cn
        br = jnp.where(is_a, 0, 1)

        g = s + LEADG
        gslot = g % NBUF
        ga = jnp.minimum(g, NA - 1)
        gb = jnp.clip(g - NA, 0, NB - 1)
        gw = jnp.maximum(g - NS, 0)

        def issue_part(u0, n):
            @pl.when(g < NA)
            def _():
                kv_issue(ka, va, ga // CA, (ga % CA) * R, gslot, u0, n)

            @pl.when(jnp.logical_and(g >= NA, g < NS))
            def _():
                kv_issue(kb, vb, gb // CB, SK - W + (gb % CB) * R, gslot, u0, n)

            @pl.when(g >= NS)
            def _():
                w_issue(1, gw * U + u0, n)

        kv_wait(slot)

        @pl.when(c == 0)
        def _():
            m_scr[...] = jnp.full(m_scr.shape, -jnp.inf, jnp.float32)
            l_scr[...] = jnp.zeros(l_scr.shape, jnp.float32)
            acc_scr[...] = jnp.zeros(acc_scr.shape, jnp.float32)

        hp = HKV // ISPLIT
        for part in range(ISPLIT):
            issue_part(part * U // ISPLIT, U // ISPLIT)
            for j in range(part * hp, (part + 1) * hp):
                sc = lax.dot_general(q_scr[br * HKV + j], kbuf[slot, j], _NT,
                                     preferred_element_type=jnp.float32)
                m_prev = m_scr[j]
                m_new = jnp.maximum(m_prev, jnp.max(sc, axis=1, keepdims=True))
                alpha = jnp.exp(m_prev - m_new)
                p = jnp.exp(sc - jnp.concatenate([m_new] * (R // 128), axis=1))
                psum = p[:, 0:128]
                for i in range(1, R // 128):
                    psum = psum + p[:, i * 128:(i + 1) * 128]
                m_scr[j] = m_new
                l_scr[j] = alpha * l_scr[j] + psum
                pv = jnp.dot(p.astype(jnp.bfloat16), vbuf[slot, j],
                             preferred_element_type=jnp.float32)
                acc_scr[j] = jnp.concatenate([alpha] * (DH // 128), axis=1) * acc_scr[j] + pv

        @pl.when(c == cn - 1)
        def _():
            for j in range(HKV):
                o = acc_scr[j] / jnp.sum(l_scr[j], axis=1, keepdims=True)
                old = lhs_scr[br, :, j * GW:(j + 1) * GW].astype(jnp.float32)
                new = jnp.concatenate(
                    [jnp.where(row == 2 * b, o, old[:, :DH]),
                     jnp.where(row == 2 * b + 1, o, old[:, DH:])], axis=1)
                lhs_scr[br, :, j * GW:(j + 1) * GW] = new.astype(jnp.bfloat16)

        return carry

    lax.fori_loop(0, NS, kv_step, 0)

    def emit(br, seg):
        y = y_scr[br * NSEG + seg]
        res = jnp.concatenate([y[0:1] + y[1:2], y[2:3] + y[3:4]], axis=0)
        res = res.astype(out_ref.dtype)
        for g in range(WG):
            o0 = br * D + g * WR + seg * SEGR
            out_ref[:, o0:o0 + SEGR] = res[:, g * SEGR:(g + 1) * SEGR]

    def pick(it, vals):
        out = jnp.int32(vals[0])
        for k in range(1, len(vals)):
            out = jnp.where(it >= k, jnp.int32(vals[k]), out)
        return out

    def issue_last():
        i0 = (NSEG - 1) * SEGR // T
        la = [(i, c) for i in range(i0, i0 + SEGR // T) for c in range(NWC)]
        lb = [(i, t * (NWC // NP) + c, t) for t in range(NP)
              for i in range(i0, i0 + SEGR // T) for c in range(NWC // NP)]
        for (ia, ca), (ib, cb, t) in zip(la, lb):
            pltpu.make_async_copy(woa.at[:, pl.ds(ia * T, T), pl.ds(ca * WC, WC)],
                                  w_buf.at[2, :, pl.ds(ia * T, T), pl.ds(ca * WC, WC)],
                                  wsem.at[3 * NSEG - 1]).start(priority=0)
            pltpu.make_async_copy(wob.at[:, pl.ds(ib * T, T), pl.ds(cb * WC, WC)],
                                  w_buf.at[3, :, pl.ds(ib * T, T), pl.ds(cb * WC, WC)],
                                  wsem.at[4 * NSEG - 1 + t]).start(priority=1)

    def o_step(it, carry):
        br = pick(it, [e[0] for e in O_SCHED[:-1]])
        seg = pick(it, [e[1] for e in O_SCHED[:-1]])
        w_wait(2 + br, seg)

        @pl.when(it < N_OI)
        def _():
            w_issue(1, LEAD + jnp.minimum(it, N_OI - 1) * OI, OI)

        @pl.when(it == N_OI)
        def _():
            issue_last()

        y_scr[br * NSEG + seg] = lax.dot_general(lhs_scr[br], w_load(2 + br, seg), _NT,
                                                 preferred_element_type=jnp.float32)

        @pl.when(it == len(O_SCHED) - 2 - N_LATE)
        def _():
            for e in O_SCHED[:-1 - N_LATE]:
                emit(*e)

        return carry

    lax.fori_loop(0, len(O_SCHED) - 1, o_step, 0)
    for e in O_SCHED[len(O_SCHED) - 1 - N_LATE:-1]:
        emit(*e)

    KP = NQ // NP
    r0 = (NSEG - 1) * SEGR

    def t_step(t, y):
        k0 = pl.multiple_of(t * KP, KP)
        v = w_buf.at[3, :, pl.ds(r0, SEGR), pl.ds(k0, KP)]
        pltpu.make_async_copy(v, v, wsem.at[4 * NSEG - 1 + t]).wait()
        blk = w_buf[3, :, pl.ds(r0, SEGR), pl.ds(k0, KP)].reshape(WG * SEGR, KP)
        return y + lax.dot_general(lhs_scr[1, :, pl.ds(k0, KP)], blk, _NT,
                                   preferred_element_type=jnp.float32)

    y_scr[2 * NSEG - 1] = lax.fori_loop(0, NP, t_step, jnp.zeros((8, WG * SEGR), jnp.float32))
    emit(*O_SCHED[-1])


@jax.jit
def pallas_concat_heads__gqa_block_cached__sliding_block_cached__decode_kernel(
    A_x: jax.Array,
    A_k_cache: jax.Array,
    A_v_cache: jax.Array,
    A_wq: jax.Array,
    A_wo: jax.Array,
    B_x: jax.Array,
    B_k_cache: jax.Array,
    B_v_cache: jax.Array,
    B_wq: jax.Array,
    B_wo: jax.Array,
):
    assert A_x.shape == B_x.shape == (B, 1, D)
    assert A_k_cache.shape == A_v_cache.shape == (B, HKV, SK, DH)
    assert B_k_cache.shape == B_v_cache.shape == (B, HKV, SK, DH)
    assert A_wq.shape == B_wq.shape == (D, NQ)
    assert A_wo.shape == B_wo.shape == (NQ, D)

    def prep(x, k, v, wq, wo):
        return (x.reshape(B, D), k, v, wq.reshape(WG, WR, NQ), wo.T.reshape(WG, WR, NQ))

    bf16, f32 = jnp.bfloat16, jnp.float32
    out = pl.pallas_call(
        _kernel,
        out_shape=jax.ShapeDtypeStruct((B, 2 * D), bf16),
        in_specs=[pl.BlockSpec(memory_space=pltpu.HBM)] * 10,
        out_specs=pl.BlockSpec(memory_space=pltpu.VMEM),
        scratch_shapes=[
            pltpu.VMEM((NBUF, HKV, R, DH), bf16),
            pltpu.VMEM((NBUF, HKV, R, DH), bf16),
            pltpu.VMEM((4, WG, WR, NQ), bf16),
            pltpu.VMEM((2, B, D), bf16),
            pltpu.VMEM((2 * NSEG, 8, WG * SEGR), bf16),
            pltpu.VMEM((2 * HKV, 8, DH), bf16),
            pltpu.VMEM((2, 8, NQ), f32),
            pltpu.VMEM((HKV, 8, 128), f32),
            pltpu.VMEM((HKV, 8, 128), f32),
            pltpu.VMEM((HKV, 8, DH), f32),
            pltpu.VMEM((2, 8, NQ), bf16),
            pltpu.VMEM((2 * NSEG, 8, WG * SEGR), f32),
            pltpu.SemaphoreType.DMA((NBUF,)),
            pltpu.SemaphoreType.DMA((NBUF,)),
            pltpu.SemaphoreType.DMA((4 * NSEG - 1 + NP,)),
            pltpu.SemaphoreType.DMA((2,)),
        ],
        compiler_params=pltpu.CompilerParams(
            vmem_limit_bytes=64 * 1024 * 1024,
            disable_bounds_checks=True,
            disable_semaphore_checks=True,
        ),
    )(*prep(A_x, A_k_cache, A_v_cache, A_wq, A_wo),
      *prep(B_x, B_k_cache, B_v_cache, B_wq, B_wo))
    return out.reshape(B, 1, 2 * D)
```
